```python
import jax
import jax.numpy as jnp

def _softmax(x, axis=-1):
    return jax.nn.softmax(x, axis=axis)
def _gelu(x):
    return jax.nn.gelu(x, approximate=True)
def _silu(x):
    return jax.nn.silu(x)
def _sigmoid(x):
    return jax.nn.sigmoid(x)
def _layernorm(x, axis=-1, eps=1e-5):
    m = jnp.mean(x, axis=axis, keepdims=True)
    v = jnp.var(x, axis=axis, keepdims=True)
    return (x - m) / jnp.sqrt(v + eps)
def _scatter_add(tgt, idx, src, axis=0):
    return tgt.at[idx].add(src)
def _segment_sum(src, seg, n):
    return jax.ops.segment_sum(src, seg, n)
class _Rng:
    def __init__(self, key):
        self._k = key
    def _next(self):
        self._k, sub = jax.random.split(self._k)
        return sub
    def normal(self, shape):
        return jax.random.normal(self._next(), shape, dtype=jnp.bfloat16)
    def randint(self, lo, hi, shape):
        return jax.random.randint(self._next(), shape, lo, hi, dtype=jnp.int32)
    def uniform(self, shape, lo=0.0, hi=1.0):
        return jax.random.uniform(self._next(), shape, jnp.bfloat16, lo, hi)
    def permutation(self, n):
        return jax.random.permutation(self._next(), n)


kernel_name = 'gated_mix__ssm_conv_h3__compressed_kv_cla__prompt'

def setup_inputs():
    _rng = _Rng(jax.random.key(int.from_bytes(__import__("os").urandom(4), "little")))
    _w = (lambda a: (lambda t: t.astype(jnp.bfloat16) if jnp.issubdtype(t.dtype, jnp.floating) else t)(jnp.asarray(a)))
    def _A_setup():
        B, S, D = 1, 2048, 1024
        ks = 4
        return {
            "q": _w((lambda *s: _rng.normal(s) * 0.05)(B, S, D)),
            "k": _w((lambda *s: _rng.normal(s) * 0.05)(B, S, D)),
            "v": _w((lambda *s: _rng.normal(s) * 0.05)(B, S, D)),
            "shift_k": _w((lambda *s: _rng.normal(s) * 0.05)(D, ks) * 0.5),
            "ssm_k": _w((lambda *s: _rng.normal(s) * 0.05)(D, S) * (1.0 / S ** 0.5)),
            "ssm_D": _w((lambda *s: _rng.normal(s) * 0.05)(D)),
        }
    _A_in = _A_setup()

    def _B_setup():
        B, H, Sq, Sk, D, M = 1, 32, 2048, 2048, 128, 1024
        Dc = 4 * D
        return {
            "x": _w((lambda *s: _rng.normal(s) * 0.05)(B, Sq, M)),
            "c_kv": _w((lambda *s: _rng.normal(s) * 0.05)(B, Sk, Dc)),
            "w_q": _w((lambda *s: _rng.normal(s) * 0.05)(M, H, D) * (M ** -0.5)),
            "w_uk": _w((lambda *s: _rng.normal(s) * 0.05)(Dc, H, D) * (Dc ** -0.5)),
            "w_uv": _w((lambda *s: _rng.normal(s) * 0.05)(Dc, H, D) * (Dc ** -0.5)),
            "w_o": _w((lambda *s: _rng.normal(s) * 0.05)(H, D, M) * ((H * D) ** -0.5)),
        }
    _B_in = _B_setup()

    return {
        "A_q": _A_in["q"],
        "A_k": _A_in["k"],
        "A_v": _A_in["v"],
        "A_shift_k": _A_in["shift_k"],
        "A_ssm_k": _A_in["ssm_k"],
        "A_ssm_D": _A_in["ssm_D"],
        "B_x": _B_in["x"],
        "B_c_kv": _B_in["c_kv"],
        "B_w_q": _B_in["w_q"],
        "B_w_uk": _B_in["w_uk"],
        "B_w_uv": _B_in["w_uv"],
        "B_w_o": _B_in["w_o"],
        "gate_w": _w((lambda *s: _rng.normal(s) * 0.05)(1024)),
    }

def reference(A_q, A_k, A_v, A_shift_k, A_ssm_k, A_ssm_D, B_x, B_c_kv, B_w_q, B_w_uk, B_w_uv, B_w_o, gate_w):
    def _A_ref(q, k, v, shift_k, ssm_k, ssm_D):
        B, S, D = q.shape
        ks = shift_k.shape[-1]
        k_pad = jnp.pad(k, ((0, 0), (ks - 1, 0), (0, 0)))
        k_shift = jnp.zeros_like(k)
        for t in range(ks):
            k_shift = k_shift + k_pad[:, t:t + S, :] * shift_k[:, ks - 1 - t][None, None, :]
        kv = k_shift * v
        L = 2 * S
        kv_pad = jnp.pad(kv, ((0, 0), (0, S), (0, 0)))
        kf_pad = jnp.pad(ssm_k, ((0, 0), (0, S)))
        kv_f = (lambda x, axes=(-2,-1): jnp.fft.rfft2(x.astype(jnp.float32), axes=axes))(kv_pad[:, None, :, :], axes=(1, 2))
        kf_f = (lambda x, axes=(-2,-1): jnp.fft.rfft2(x.astype(jnp.float32), axes=axes))(kf_pad[:, None, :], axes=(1, 2))
        kf_f = (lambda x, *d: x.transpose(*d))(kf_f, 1, 2, 0)
        y_f = kv_f * kf_f[None, :, :, :]
        y = (lambda x, s, axes=(-2,-1): jnp.fft.irfft2(x, s=s, axes=axes).astype(jnp.bfloat16))(y_f, (1, L), axes=(1, 2))[:, 0, :S, :]
        y = y + kv * ssm_D[None, None, :]
        return q * y

    def _B_ref(x, c_kv, w_q, w_uk, w_uv, w_o):
        B, Sq, M = x.shape[0], x.shape[1], x.shape[2]
        Sk = c_kv.shape[1]
        H, D = w_q.shape[1], w_q.shape[2]
        q = jnp.einsum("bqm,mhd->bhqd", x, w_q)
        k = jnp.einsum("bkc,chd->bhkd", c_kv, w_uk)
        v = jnp.einsum("bkc,chd->bhkd", c_kv, w_uv)
        scores = jnp.einsum("bhqd,bhkd->bhqk", q, k) * (D ** -0.5)
        off = Sk - Sq
        qi = jnp.arange(Sq)[:, None]
        kj = jnp.arange(Sk)[None, :]
        cmask = kj <= (qi + off)
        scores = jnp.where(cmask[None, None], scores, -1e9)
        p = _softmax(scores, axis=-1)
        ctx = jnp.einsum("bhqk,bhkd->bhqd", p, v)
        return jnp.einsum("bhqd,hdm->bqm", ctx, w_o)

    x = A_q
    g = _sigmoid((x * gate_w).sum(-1, keepdims=True))
    a = _A_ref(x, A_k, A_v, A_shift_k, A_ssm_k, A_ssm_D)
    b = _B_ref(x, B_c_kv, B_w_q, B_w_uk, B_w_uv, B_w_o)
    return g * a + (1 - g) * b
```

```python
import functools
import math

import jax
import jax.numpy as jnp
import numpy as np
from jax import lax
import jax.experimental.pallas as pl
import jax.experimental.pallas.tpu as pltpu

F32 = jnp.float32
BF16 = jnp.bfloat16
U32 = jnp.uint32

S = 2048
DM = 1024
H = 32
DH = 128
DC = 512
KS = 4
TB = 128
NB = S // TB
CT = 128
BQ = 256
RB = 256
PM = 512


def _dft_matrices():
    k = np.concatenate([np.arange(0, TB, 2), np.arange(1, TB, 2)]).astype(np.float64)
    t = np.arange(TB, dtype=np.float64)
    ang = 2.0 * np.pi * np.outer(k + 0.5, t) / (2 * TB)
    fwd = np.concatenate([np.cos(ang), -np.sin(ang)], axis=0)
    inv = fwd.T / TB
    return fwd.astype(np.float32), inv.astype(np.float32)


_FWD, _INV = _dft_matrices()


def _dot(a, b):
    return jnp.dot(a, b, preferred_element_type=F32)


def _dot_nt(a, b):
    return lax.dot_general(a, b, (((1,), (1,)), ((), ())), preferred_element_type=F32)


def _head_pair(w_ref, group, pair, rows):
    span = rows * (H // 2) - 12
    w32 = w_ref.bitcast(U32).at[pl.ds(pl.multiple_of(4 * group, 4), span)]
    w = w32[pl.ds(pair, rows, stride=H // 2), :]
    lo = lax.bitcast_convert_type(w << 16, F32)
    hi = lax.bitcast_convert_type(w & jnp.uint32(0xFFFF0000), F32)
    return lo.astype(BF16), hi.astype(BF16)


def _causal_conv(x_ref, g_ref, part, rows, lo, hi):
    out = []
    for i in range(lo, hi):
        acc = None
        for j in range(i + 1):
            t = x_ref[part, i - j, rows, :] * g_ref[part, j, rows, :]
            acc = t if acc is None else acc + t
        out.append(acc)
    return out


def _kernel(
    aq_hbm, ak_hbm, av_hbm, shift_ref, ssmk_hbm, ssmd_ref, c_hbm,
    wq_hbm, wuk_hbm, wuv_hbm, wo_hbm, gw_ref, fwd_ref, inv_ref,
    out_hbm,
    aq_v, ak_v, av_v, ssmk_v, c_v, wq_v, wuk_v, wuv_v, wo_v,
    wkv_v, wqs_v, q_v, k_v, v_v, y_v, kv_v, xs_v, hs_v, gs_v, ys_v, o_v, in_sem, out_sem,
):
    srcs = (c_hbm, wuk_hbm, wuv_hbm, aq_hbm, wq_hbm, ak_hbm, av_hbm, ssmk_hbm, wo_hbm)
    dsts = (c_v, wuk_v, wuv_v, aq_v, wq_v, ak_v, av_v, ssmk_v, wo_v)
    cps = [pltpu.make_async_copy(s, d, in_sem.at[i]) for i, (s, d) in enumerate(zip(srcs, dsts))]
    for cp in cps[:3]:
        cp.start()
    for cp in cps[:3]:
        cp.wait()
    for cp in cps[3:]:
        cp.start()

    def kv_group(group, carry):
        for pair in range(4):
            k0, k1 = _head_pair(wuk_v, group, pair, DC)
            v0, v1 = _head_pair(wuv_v, group, pair, DC)
            wkv_v[pair] = jnp.concatenate([k0, k1, v0, v1], axis=1)

        def kv_proj(pair, carry):
            w = wkv_v[pair]
            h0 = 8 * group + 2 * pair
            for r in range(S // PM):
                rows = slice(r * PM, (r + 1) * PM)
                o = _dot(c_v[rows, :], w).astype(BF16)
                k_v[h0, rows, :] = o[:, 0 * DH:1 * DH]
                k_v[h0 + 1, rows, :] = o[:, 1 * DH:2 * DH]
                v_v[h0, rows, :] = o[:, 2 * DH:3 * DH]
                v_v[h0 + 1, rows, :] = o[:, 3 * DH:4 * DH]
            return carry

        return lax.fori_loop(0, 4, kv_proj, carry)

    lax.fori_loop(0, H // 8, kv_group, 0)

    for cp in cps[3:8]:
        cp.wait()

    qscale = DH ** -0.5 * math.log2(math.e)

    def q_proj_and_conv(ct, carry):
        ch = pl.ds(pl.multiple_of(ct * CT, CT), CT)
        sh = shift_ref[:, ch].astype(F32)
        kf = ak_v[:, ch].astype(F32)
        t_idx = lax.broadcasted_iota(jnp.int32, (S, CT), 0)
        ksh = kf * sh[0:1, :]
        for j in range(1, KS):
            ksh = ksh + jnp.where(t_idx >= j, pltpu.roll(kf, j, 0), 0.0) * sh[j:j + 1, :]
        kv_v[...] = (ksh * av_v[:, ch].astype(F32)).astype(BF16)
        fwd = fwd_ref[...]
        for i in range(NB):
            xf = _dot(fwd, kv_v[i * TB:(i + 1) * TB, :])
            xs_v[0, i] = xf[:TB] + xf[TB:]
            xs_v[1, i] = xf[:TB]
            xs_v[2, i] = xf[TB:]
            hs_v[i] = _dot_nt(fwd, ssmk_v[ch, i * TB:(i + 1) * TB])

        w = wqs_v[ct % 2]

        def q_chunk(r):
            rows = slice(r * PM, (r + 1) * PM)
            o = (_dot(aq_v[rows, :], w) * qscale).astype(BF16)
            for n in range(4):
                q_v[4 * ct + n, rows, :] = o[:, n * DH:(n + 1) * DH]

        def bins(f):
            rows = slice(8 * f, 8 * f + 8)
            rim = slice(TB + 8 * f, TB + 8 * f + 8)
            even = f < TB // 16
            for j in range(NB):
                gr, gi = hs_v[j, rows, :], hs_v[j, rim, :]
                if j:
                    pr, pi = hs_v[j - 1, rows, :], hs_v[j - 1, rim, :]
                    gr, gi = (gr - pi, gi + pr) if even else (gr + pi, gi - pr)
                gs_v[0, j, rows, :] = gr
                gs_v[1, j, rows, :] = gi - gr
                gs_v[2, j, rows, :] = gi + gr
            for lo in range(0, NB, 4):
                s1 = _causal_conv(xs_v, gs_v, 0, rows, lo, lo + 4)
                s2 = _causal_conv(xs_v, gs_v, 1, rows, lo, lo + 4)
                s3 = _causal_conv(xs_v, gs_v, 2, rows, lo, lo + 4)
                for n in range(4):
                    ys_v[lo + n, rows, :] = s1[n] - s3[n]
                    ys_v[lo + n, rim, :] = s1[n] + s2[n]

        nch = S // PM
        per = (TB // 8) // nch
        for r in range(nch):
            q_chunk(r)
            for f in range(r * per, (r + 1) * per):
                bins(f)

        inv = inv_ref[...]
        d = ssmd_ref[:, ch].astype(F32)
        for i in range(NB):
            rows = slice(i * TB, (i + 1) * TB)
            y = _dot(inv, ys_v[i].astype(BF16))
            y_v[rows, ch] = (y + kv_v[rows, :].astype(F32) * d).astype(BF16)
        return carry

    def q_group(group, carry):
        for half in range(2):
            qa, qb = _head_pair(wq_v, group, 2 * half, DM)
            qc, qd = _head_pair(wq_v, group, 2 * half + 1, DM)
            wqs_v[half] = jnp.concatenate([qa, qb, qc, qd], axis=1)
        return lax.fori_loop(2 * group, 2 * group + 2, q_proj_and_conv, carry)

    lax.fori_loop(0, H // 8, q_group, 0)

    def attend(h, carry):
        nq = S // BQ
        tri = (lax.broadcasted_iota(jnp.int32, (BQ, BQ), 1)
               <= lax.broadcasted_iota(jnp.int32, (BQ, BQ), 0))

        def scores(i):
            return _dot_nt(q_v[h, i * BQ:(i + 1) * BQ, :], k_v[h, 0:(i + 1) * BQ, :])

        s_next = scores(0)
        for i in range(nq):
            s = s_next
            if i + 1 < nq:
                s_next = scores(i + 1)
            diag = jnp.where(tri, s[:, i * BQ:], -1e9)
            s = jnp.concatenate([s[:, :i * BQ], diag], axis=1) if i else diag
            p = jnp.exp2(s - jnp.max(s, axis=1, keepdims=True))
            l = jnp.sum(p, axis=1, keepdims=True)
            o = _dot(p.astype(BF16), v_v[h, 0:(i + 1) * BQ, :])
            q_v[h, i * BQ:(i + 1) * BQ, :] = (o / l).astype(BF16)
        return carry

    lax.fori_loop(0, H, attend, 0)

    for cp in cps[8:]:
        cp.wait()

    def out_copy(r):
        return pltpu.make_async_copy(
            o_v.at[r], out_hbm.at[pl.ds(r * RB, RB), :], out_sem.at[r])

    def out_proj(r, carry):
        rows = pl.ds(pl.multiple_of(r * RB, RB), RB)
        ctx = jnp.concatenate([q_v[n, rows, :] for n in range(H)], axis=1)
        b = _dot(ctx, wo_v[...])
        aq = aq_v[rows, :].astype(F32)
        g = jax.nn.sigmoid(jnp.sum(aq * gw_ref[...].astype(F32), axis=1, keepdims=True))
        a = aq * y_v[rows, :].astype(F32)
        o_v[r] = (g * a + (1.0 - g) * b).astype(BF16)
        out_copy(r).start()
        return carry

    lax.fori_loop(0, S // RB, out_proj, 0)
    for r in range(S // RB):
        out_copy(r).wait()


@jax.jit
def pallas_gated_mix__ssm_conv_h3__compressed_kv_cla__prompt_kernel(
    A_q: jax.Array,
    A_k: jax.Array,
    A_v: jax.Array,
    A_shift_k: jax.Array,
    A_ssm_k: jax.Array,
    A_ssm_D: jax.Array,
    B_x: jax.Array,
    B_c_kv: jax.Array,
    B_w_q: jax.Array,
    B_w_uk: jax.Array,
    B_w_uv: jax.Array,
    B_w_o: jax.Array,
    gate_w: jax.Array,
):
    hbm = pl.BlockSpec(memory_space=pl.ANY)
    vmem = pl.BlockSpec(memory_space=pltpu.VMEM)
    out = pl.pallas_call(
        _kernel,
        out_shape=jax.ShapeDtypeStruct((S, DM), BF16),
        in_specs=[hbm, hbm, hbm, vmem, hbm, vmem, hbm, hbm, hbm, hbm, hbm, vmem, vmem, vmem],
        out_specs=hbm,
        scratch_shapes=[
            pltpu.VMEM((S, DM), BF16),
            pltpu.VMEM((S, DM), BF16),
            pltpu.VMEM((S, DM), BF16),
            pltpu.VMEM((DM, S), BF16),
            pltpu.VMEM((S, DC), BF16),
            pltpu.VMEM((DM * H, DH), BF16),
            pltpu.VMEM((DC * H, DH), BF16),
            pltpu.VMEM((DC * H, DH), BF16),
            pltpu.VMEM((H * DH, DM), BF16),
            pltpu.VMEM((4, DC, 4 * DH), BF16),
            pltpu.VMEM((2, DM, 4 * DH), BF16),
            pltpu.VMEM((H, S, DH), BF16),
            pltpu.VMEM((H, S, DH), BF16),
            pltpu.VMEM((H, S, DH), BF16),
            pltpu.VMEM((S, DM), BF16),
            pltpu.VMEM((S, CT), BF16),
            pltpu.VMEM((3, NB, TB, CT), F32),
            pltpu.VMEM((NB, 2 * TB, CT), F32),
            pltpu.VMEM((3, NB, TB, CT), F32),
            pltpu.VMEM((NB, 2 * TB, CT), F32),
            pltpu.VMEM((S // RB, RB, DM), BF16),
            pltpu.SemaphoreType.DMA((9,)),
            pltpu.SemaphoreType.DMA((S // RB,)),
        ],
        compiler_params=pltpu.CompilerParams(vmem_limit_bytes=126 * 2**20),
        name="gated_mix_h3_cla",
    )(
        A_q.reshape(S, DM), A_k.reshape(S, DM), A_v.reshape(S, DM),
        A_shift_k.T, A_ssm_k, A_ssm_D.reshape(1, DM),
        B_c_kv.reshape(S, DC),
        B_w_q.reshape(DM * H, DH), B_w_uk.reshape(DC * H, DH), B_w_uv.reshape(DC * H, DH),
        B_w_o.reshape(H * DH, DM), gate_w.reshape(1, DM),
        jnp.asarray(_FWD, BF16), jnp.asarray(_INV, BF16),
    )
    return out.reshape(1, S, DM)
```

```python
import functools
import math

import jax
import jax.numpy as jnp
import numpy as np
from jax import lax
import jax.experimental.pallas as pl
import jax.experimental.pallas.tpu as pltpu

F32 = jnp.float32
BF16 = jnp.bfloat16
U32 = jnp.uint32

S = 2048
DM = 1024
H = 32
DH = 128
DC = 512
KS = 4
T = 128
NB = S // T
NC = DM // T
PM = 256
RB = 256
QK_TILES = 4
PV_TILES = 2
XS, GS, YS = 0, 3 * NB, 5 * NB
HALO = 16


def _dft_matrices():
    k = np.concatenate([np.arange(0, T, 2), np.arange(1, T, 2)]).astype(np.float64)
    t = np.arange(T, dtype=np.float64)
    ang = 2.0 * np.pi * np.outer(k + 0.5, t) / (2 * T)
    fwd = np.concatenate([np.cos(ang), -np.sin(ang)], axis=0)
    inv = fwd.T / T
    return fwd.astype(np.float32), inv.astype(np.float32)


_FWD, _INV = _dft_matrices()


def _dot(a, b):
    return jnp.dot(a, b, preferred_element_type=F32)


def _dot_nt(a, b):
    return lax.dot_general(a, b, (((1,), (1,)), ((), ())), preferred_element_type=F32)


def _split_heads(w):
    lo = lax.bitcast_convert_type(w << 16, F32)
    hi = lax.bitcast_convert_type(w & jnp.uint32(0xFFFF0000), F32)
    return lo.astype(BF16), hi.astype(BF16)


def _finish(gen):
    for _ in gen:
        pass


def _interleave(*streams):
    steps = [((n + 0.5 * (k > 0)) / len(st), k, fn)
             for k, st in enumerate(streams) for n, fn in enumerate(st)]
    for _, _, fn in sorted(steps, key=lambda t: t[:2]):
        fn()


def _kernel(
    zero_ref, aq_hbm, ak_hbm, av_hbm, shift_ref, ssmk_hbm, ssmd_ref, c_hbm,
    wq_hbm, wuk_hbm, wuv_hbm, wo_hbm, gw_ref, fwd_ref, inv_ref,
    out_hbm,
    aq_v, ak_v, av_v, ssmk_v, c_v, wq_raw, wuk_raw, wuv_raw, wo_v,
    w_v, q_v, k_v, v_v, y_v, kv_v, spec_v, o_v,
    x_sem, wq_sem, conv_sem, wkv_sem, misc_sem, out_sem,
):
    XC = 4
    xr = S // XC
    wr = DC // NC

    def aligned(i, n):
        return pl.ds(i * n if isinstance(i, int) else pl.multiple_of(i * n, n), n)

    def x_copy(r):
        rows = pl.ds(r * xr, xr)
        return pltpu.make_async_copy(aq_hbm.at[rows], aq_v.at[rows], x_sem.at[r])

    def wq_copy(g):
        pairs = H // 4
        return pltpu.make_async_copy(
            wq_hbm.bitcast(U32).at[:, pl.ds(g * pairs, pairs), :],
            wq_raw.at[g].reshape(DM, pairs, DH), wq_sem.at[g])

    def conv_copies(ct):
        ch = aligned(ct, T)
        return (
            pltpu.make_async_copy(ak_hbm.at[:, ch], ak_v.at[ct, pl.ds(HALO, S)], conv_sem.at[3 * ct]),
            pltpu.make_async_copy(av_hbm.at[:, ch], av_v.at[ct], conv_sem.at[3 * ct + 1]),
            pltpu.make_async_copy(ssmk_hbm.at[ch], ssmk_v.at[ct], conv_sem.at[3 * ct + 2]),
        )

    def wkv_copies(ct):
        pairs = H // 4
        return tuple(
            pltpu.make_async_copy(
                src.bitcast(U32).at[aligned(ct, wr), pl.ds(g * pairs, pairs), :],
                dst.at[ct, g].reshape(wr, pairs, DH), wkv_sem.at[4 * ct + 2 * n + g])
            for n, (src, dst) in enumerate(((wuk_hbm, wuk_raw), (wuv_hbm, wuv_raw)))
            for g in range(2))

    c_copy = pltpu.make_async_copy(c_hbm, c_v, misc_sem.at[0])
    wo_copy = pltpu.make_async_copy(wo_hbm, wo_v, misc_sem.at[1])

    wq_copy(0).start()
    x_copy(0).start()

    ak_v[:, 0:HALO, :] = jnp.zeros((NC, HALO, T), BF16)

    qscale = DH ** -0.5 * math.log2(math.e)
    zero = zero_ref[0]

    def unpack_wq(pair, part):
        g, p = divmod(pair, H // 4)
        lo, hi = _split_heads(wq_raw[g, pl.ds(part * T * (H // 4) + p, T, stride=H // 4), :])
        w_v[zero + 2 * pair, part * T:(part + 1) * T, :] = lo
        w_v[zero + 2 * pair + 1, part * T:(part + 1) * T, :] = hi

    def unpack_wkv(ct, pair):
        k_rows, v_rows = aligned(DM // wr + ct, wr), aligned((DM + DC) // wr + ct, wr)
        g, p = divmod(pair, H // 4)
        k0, k1 = _split_heads(wuk_raw[ct, g, pl.ds(p, wr, stride=H // 4), :])
        v0, v1 = _split_heads(wuv_raw[ct, g, pl.ds(p, wr, stride=H // 4), :])
        w_v[2 * pair, k_rows, :] = k0
        w_v[2 * pair + 1, k_rows, :] = k1
        w_v[2 * pair, v_rows, :] = v0
        w_v[2 * pair + 1, v_rows, :] = v1

    def q_proj(h, r, n):
        rows = aligned(r, n)
        q_v[h, rows, :] = (_dot(aq_v[rows, :], w_v[h, :DM, :]) * qscale).astype(BF16)

    def k_proj(h, r):
        rows = slice(r * PM, (r + 1) * PM)
        k_v[rows, :] = _dot(c_v[rows, :], w_v[h, DM:DM + DC, :]).astype(BF16)

    def v_proj(h, r):
        rows = slice(r * PM, (r + 1) * PM)
        v_v[rows, :] = _dot(c_v[rows, :], w_v[h, DM + DC:, :]).astype(BF16)

    def conv_input(ct, i):
        sh = shift_ref[:, aligned(ct, T)].astype(F32)
        kf = ak_v[ct, i * T:(i + 1) * T + HALO, :].astype(F32)
        ksh = kf * sh[0:1, :]
        for j in range(1, KS):
            ksh = ksh + pltpu.roll(kf, j, 0) * sh[j:j + 1, :]
        rows = slice(i * T, (i + 1) * T)
        kv_v[rows, :] = (ksh[HALO:] * av_v[ct, rows, :].astype(F32)).astype(BF16)

    def input_spectrum(i):
        xf = _dot(fwd_ref[...], kv_v[i * T:(i + 1) * T, :])
        spec_v[XS + i] = xf[:T] + xf[T:]
        spec_v[XS + NB + i] = xf[:T]
        spec_v[XS + 2 * NB + i] = xf[T:]

    def kernel_spectrum(ct, i, prev):
        half = T // 2
        hf = _dot_nt(fwd_ref[...], ssmk_v[ct, :, i * T:(i + 1) * T])
        gr, gi = hf[:T], hf[T:]
        if i:
            pr, pi = prev[0][:T], prev[0][T:]
            gr = jnp.concatenate([gr[:half] - pi[:half], gr[half:] + pi[half:]], axis=0)
            gi = jnp.concatenate([gi[:half] + pr[:half], gi[half:] - pr[half:]], axis=0)
        prev[0] = hf
        spec_v[GS + i] = gr
        spec_v[GS + NB + i] = gi

    def conv_bins(lo, hi, f):
        rows = slice(8 * f, 8 * f + 8)

        def part(n):
            outs = [None] * (hi - lo)
            for j in range(hi):
                g = spec_v[GS + j, rows, :]
                if n:
                    gi = spec_v[GS + NB + j, rows, :]
                    g = gi - g if n == 1 else gi + g
                for i in range(max(lo, j), hi):
                    t = spec_v[XS + n * NB + i - j, rows, :] * g
                    outs[i - lo] = t if j == 0 else outs[i - lo] + t
            return outs

        s1 = part(0)
        re = [a - b for a, b in zip(s1, part(2))]
        im = [a + b for a, b in zip(s1, part(1))]
        base = YS + (zero if f % 4 == 3 else 0)
        for i in range(lo, hi):
            spec_v[base + 2 * i, rows, :] = re[i - lo]
            spec_v[base + 2 * i + 1, rows, :] = im[i - lo]

    def conv_inverse(ct, i):
        d = ssmd_ref[:, aligned(ct, T)].astype(F32)
        rows = slice(i * T, (i + 1) * T)
        yf = jnp.concatenate([spec_v[YS + 2 * i], spec_v[YS + 2 * i + 1]], axis=0)
        y = _dot(inv_ref[...], yf.astype(BF16))
        y_v[ct, rows, :] = (y + kv_v[rows, :].astype(F32) * d).astype(BF16)

    def conv_tile(ct, fillers, slots):
        P = functools.partial
        fillers = iter(fillers)
        prev = [None]
        take = lambda n: [next(fillers) for _ in range(n)]
        blocks = lambda r: range(4 * r, 4 * r + 4)
        for r in range(-1, 4):
            side = [P(conv_inverse, ct, i) for i in blocks(r - 1)] if r > 0 else []
            if r < 3:
                side += [P(conv_input, ct, i) for i in blocks(r + 1)]
                for i in blocks(r + 1):
                    side += [P(input_spectrum, i), P(kernel_spectrum, ct, i, prev)]
            bins = [P(conv_bins, 4 * r, 4 * r + 4, f) for f in range(T // 8)] if r >= 0 else []
            unpack = [P(unpack_wkv, ct, pair) for pair in blocks(r)] if r >= 0 else []
            _interleave(take(slots[r + 1]), bins, side, unpack)
        _interleave([P(conv_inverse, ct, i) for i in blocks(3)], list(fillers))

    after_x = (
        (x_copy(1), x_copy(2)),
        (x_copy(3), wq_copy(1)),
        (),
        conv_copies(0) + wkv_copies(0),
    )
    unpack = (range(2, 4), range(4, 8), range(0), range(8, 16))
    wq_copy(0).wait()
    for pair in range(2):
        for part in range(DM // T):
            unpack_wq(pair, part)
    for xc in range(XC):
        x_copy(xc).wait()
        if xc == XC - 1:
            wq_copy(1).wait()
        for cp in after_x[xc]:
            cp.start()
        _interleave(
            [functools.partial(q_proj, h, r, T)
             for r in range(xc * xr // T, (xc + 1) * xr // T) for h in range(4)],
            [functools.partial(unpack_wq, pair, part)
             for pair in unpack[xc] for part in range(DM // T)])
    c_copy.start()
    done = 4 * (S // PM)
    per_tile = (H * (S // PM) - done) // NC

    def q_step(ct, carry):
        for cp in conv_copies(ct) + wkv_copies(ct):
            cp.wait()

        @pl.when(ct + 1 < NC)
        def _():
            for cp in conv_copies(ct + 1) + wkv_copies(ct + 1):
                cp.start()

        pieces = [done + per_tile * ct + n for n in range(per_tile)]
        conv_tile(ct, [functools.partial(q_proj, p // (S // PM), p % (S // PM), PM)
                       for p in pieces], (2, 4, 6, 7, 8))
        return carry

    lax.fori_loop(0, NC, q_step, 0)
    c_copy.wait()
    wo_copy.start()
    for r in range(S // PM):
        k_proj(0, r)
        v_proj(0, r)

    def attend(h, next_head):
        tri = (lax.broadcasted_iota(jnp.int32, (T, T), 1)
               <= lax.broadcasted_iota(jnp.int32, (T, T), 0))

        def scores(i, st):
            q = q_v[h, i * T:(i + 1) * T, :]
            tiles, mx = [], None
            for c0 in range(0, i + 1, QK_TILES):
                c1 = min(c0 + QK_TILES, i + 1)
                s = _dot_nt(q, k_v[c0 * T:c1 * T, :])
                for j in range(c0, c1):
                    t = s[:, (j - c0) * T:(j - c0 + 1) * T]
                    if j == i:
                        t = jnp.where(tri, t, -1e9)
                    tiles.append(t)
                    mx = t if mx is None else jnp.maximum(mx, t)
                if c1 == i + 1:
                    st["m"] = jnp.max(mx, axis=1, keepdims=True)
                    st["tiles"] = tiles
                yield

        def context(i, st):
            m, tiles = st["m"], st["tiles"]
            o = l = None
            for c0 in range(0, i + 1, PV_TILES):
                c1 = min(c0 + PV_TILES, i + 1)
                ps = [jnp.exp2(t - m) for t in tiles[c0:c1]]
                for p in ps:
                    l = p if l is None else l + p
                if c1 > 1:
                    ps[-1] = jnp.minimum(ps[-1], l)
                pc = jnp.concatenate(ps, axis=1).astype(BF16)
                oc = _dot(pc, v_v[c0 * T:c1 * T, :])
                o = oc if o is None else o + oc
                if c1 == i + 1:
                    l = jnp.sum(l, axis=1, keepdims=True)
                    r = pl.reciprocal(l, approx=True)
                    r = r * (2.0 - l * r)
                    q_v[h, i * T:(i + 1) * T, :] = (o * r).astype(BF16)
                yield

        prev = None
        for i in range(NB - 1, -1, -1):
            st = {}
            cur = scores(i, st)
            if prev is not None:
                for _ in prev:
                    next(cur, None)
                if next_head is not None and i + 1 < S // PM:
                    k_proj(next_head, i + 1)
                    v_proj(next_head, i + 1)
            _finish(cur)
            prev = context(i, st)
        _finish(prev)
        if next_head is not None:
            k_proj(next_head, 0)
            v_proj(next_head, 0)

    def attend_step(h, carry):
        attend(h, h + 1)
        return carry

    lax.fori_loop(0, H - 1, attend_step, 0)
    attend(H - 1, None)

    wo_copy.wait()

    def out_copy(r):
        return pltpu.make_async_copy(
            o_v.at[r], out_hbm.at[pl.ds(r * RB, RB), :], out_sem.at[r])

    def out_proj(r, carry):
        rows = pl.ds(pl.multiple_of(r * RB, RB), RB)
        ctx = jnp.concatenate([q_v[n, rows, :] for n in range(H)], axis=1)
        b = _dot(ctx, wo_v[...])
        aq = aq_v[rows, :].astype(F32)
        g = jax.nn.sigmoid(jnp.sum(aq * gw_ref[...].astype(F32), axis=1, keepdims=True))
        y = jnp.concatenate([y_v[n, rows, :].astype(F32) for n in range(NC)], axis=1)
        o_v[r] = (g * (aq * y) + (1.0 - g) * b).astype(BF16)
        out_copy(r).start()
        return carry

    lax.fori_loop(0, S // RB, out_proj, 0)
    for r in range(S // RB):
        out_copy(r).wait()


@jax.jit
def pallas_gated_mix__ssm_conv_h3__compressed_kv_cla__prompt_kernel(
    A_q: jax.Array,
    A_k: jax.Array,
    A_v: jax.Array,
    A_shift_k: jax.Array,
    A_ssm_k: jax.Array,
    A_ssm_D: jax.Array,
    B_x: jax.Array,
    B_c_kv: jax.Array,
    B_w_q: jax.Array,
    B_w_uk: jax.Array,
    B_w_uv: jax.Array,
    B_w_o: jax.Array,
    gate_w: jax.Array,
):
    del B_x
    hbm = pl.BlockSpec(memory_space=pl.ANY)
    vmem = pl.BlockSpec(memory_space=pltpu.VMEM)
    out = pl.pallas_call(
        _kernel,
        out_shape=jax.ShapeDtypeStruct((S, DM), BF16),
        in_specs=[pl.BlockSpec(memory_space=pltpu.SMEM), hbm, hbm, hbm, vmem, hbm, vmem, hbm, hbm, hbm, hbm, hbm, vmem, vmem, vmem],
        out_specs=hbm,
        scratch_shapes=[
            pltpu.VMEM((S, DM), BF16),
            pltpu.VMEM((NC, S + HALO, T), BF16),
            pltpu.VMEM((NC, S, T), BF16),
            pltpu.VMEM((NC, T, S), BF16),
            pltpu.VMEM((S, DC), BF16),
            pltpu.VMEM((2, DM * H // 4, DH), U32),
            pltpu.VMEM((NC, 2, DC // NC * H // 4, DH), U32),
            pltpu.VMEM((NC, 2, DC // NC * H // 4, DH), U32),
            pltpu.VMEM((H * DH, DM), BF16),
            pltpu.VMEM((H, DM + 2 * DC, DH), BF16),
            pltpu.VMEM((H, S, DH), BF16),
            pltpu.VMEM((S, DH), BF16),
            pltpu.VMEM((S, DH), BF16),
            pltpu.VMEM((NC, S, T), BF16),
            pltpu.VMEM((S, T), BF16),
            pltpu.VMEM((7 * NB, T, T), F32),
            pltpu.VMEM((S // RB, RB, DM), BF16),
            pltpu.SemaphoreType.DMA((4,)),
            pltpu.SemaphoreType.DMA((2,)),
            pltpu.SemaphoreType.DMA((3 * NC,)),
            pltpu.SemaphoreType.DMA((4 * NC,)),
            pltpu.SemaphoreType.DMA((2,)),
            pltpu.SemaphoreType.DMA((S // RB,)),
        ],
        compiler_params=pltpu.CompilerParams(vmem_limit_bytes=126 * 2**20),
        name="gated_mix_h3_cla",
    )(
        jnp.zeros((1,), jnp.int32),
        A_q.reshape(S, DM), A_k.reshape(S, DM), A_v.reshape(S, DM),
        A_shift_k.T, A_ssm_k, A_ssm_D.reshape(1, DM),
        B_c_kv.reshape(S, DC),
        B_w_q, B_w_uk, B_w_uv,
        B_w_o.reshape(H * DH, DM), gate_w.reshape(1, DM),
        jnp.asarray(_FWD, BF16), jnp.asarray(_INV, BF16),
    )
    return out.reshape(1, S, DM)
```

```python
import functools
import math

import jax
import jax.numpy as jnp
import numpy as np
from jax import lax
import jax.experimental.pallas as pl
import jax.experimental.pallas.tpu as pltpu

F32 = jnp.float32
BF16 = jnp.bfloat16
U32 = jnp.uint32

S = 2048
DM = 1024
H = 32
DH = 128
DC = 512
KS = 4
T = 128
NB = S // T
NC = DM // T
PM = 256
RB = 256
QK_TILES = 4
PV_TILES = 2
X_EDGES = (0, 128, 384, 768, S)
XS, GS, YS = 0, 3 * NB, 5 * NB
HALO = 16


def _dft_matrices():
    k = np.concatenate([np.arange(0, T, 2), np.arange(1, T, 2)]).astype(np.float64)
    t = np.arange(T, dtype=np.float64)
    ang = 2.0 * np.pi * np.outer(k + 0.5, t) / (2 * T)
    fwd = np.concatenate([np.cos(ang), -np.sin(ang)], axis=0)
    inv = fwd.T / T
    return fwd.astype(np.float32), inv.astype(np.float32)


_FWD, _INV = _dft_matrices()


def _dot(a, b):
    return jnp.dot(a, b, preferred_element_type=F32)


def _dot_nt(a, b):
    return lax.dot_general(a, b, (((1,), (1,)), ((), ())), preferred_element_type=F32)


def _split_heads(w):
    lo = lax.bitcast_convert_type(w << 16, F32)
    hi = lax.bitcast_convert_type(w & jnp.uint32(0xFFFF0000), F32)
    return lo.astype(BF16), hi.astype(BF16)


def _finish(gen):
    for _ in gen:
        pass


def _interleave(*streams):
    steps = [((n + 0.5 * (k > 0)) / len(st), k, fn)
             for k, st in enumerate(streams) for n, fn in enumerate(st)]
    for _, _, fn in sorted(steps, key=lambda t: t[:2]):
        fn()


def _kernel(
    aq_hbm, ak_hbm, av_hbm, ssmk_hbm, c_hbm, wq_hbm, wuk_hbm, wuv_hbm, wo_hbm,
    zero_hbm, shift_hbm, ssmd_hbm, gw_hbm, fwd_hbm, inv_hbm,
    out_hbm,
    aq_v, ak_v, av_v, ssmk_v, c_v, wq_raw, wuk_raw, wuv_raw, wo_v,
    w_v, q_v, k_v, v_v, y_v, kv_v, spec_v, o_v,
    fwd_ref, inv_ref, shift_ref, ssmd_ref, gw_ref, ssmd_v, zero_ref,
    small_sem, x_sem, wq_sem, conv_sem, wkv_sem, misc_sem, out_sem,
):
    wr = DC // NC

    def aligned(i, n):
        return pl.ds(i * n if isinstance(i, int) else pl.multiple_of(i * n, n), n)

    def x_copy(n):
        rows = pl.ds(X_EDGES[n], X_EDGES[n + 1] - X_EDGES[n])
        return pltpu.make_async_copy(aq_hbm.at[rows], aq_v.at[rows], x_sem.at[n])

    def wq_copy(g):
        pairs = H // 4
        return pltpu.make_async_copy(
            wq_hbm.bitcast(U32).at[:, pl.ds(g * pairs, pairs), :],
            wq_raw.at[g].reshape(DM, pairs, DH), wq_sem.at[g])

    def conv_copies(ct):
        ch = aligned(ct, T)
        return (
            pltpu.make_async_copy(ak_hbm.at[:, ch], ak_v.at[ct, pl.ds(HALO, S)], conv_sem.at[3 * ct]),
            pltpu.make_async_copy(av_hbm.at[:, ch], av_v.at[ct], conv_sem.at[3 * ct + 1]),
            pltpu.make_async_copy(ssmk_hbm.at[ch], ssmk_v.at[ct], conv_sem.at[3 * ct + 2]),
        )

    def wkv_copies(ct):
        pairs = H // 4
        return tuple(
            pltpu.make_async_copy(
                src.bitcast(U32).at[aligned(ct, wr), pl.ds(g * pairs, pairs), :],
                dst.at[ct, g].reshape(wr, pairs, DH), wkv_sem.at[4 * ct + 2 * n + g])
            for n, (src, dst) in enumerate(((wuk_hbm, wuk_raw), (wuv_hbm, wuv_raw)))
            for g in range(2))

    c_copy = pltpu.make_async_copy(c_hbm, c_v, misc_sem.at[0])
    wo_copy = pltpu.make_async_copy(wo_hbm, wo_v, misc_sem.at[1])

    small_copies = [
        pltpu.make_async_copy(src, dst, small_sem.at[n]) for n, (src, dst) in enumerate((
            (shift_hbm, shift_ref), (ssmd_hbm, ssmd_ref), (gw_hbm, gw_ref),
            (fwd_hbm, fwd_ref), (inv_hbm, inv_ref)))]
    zero_copy = pltpu.make_async_copy(zero_hbm, zero_ref, misc_sem.at[2])

    zero_copy.start()
    wq_copy(0).start()
    x_copy(0).start()
    zero_copy.wait()

    ak_v[:, 0:HALO, :] = jnp.zeros((NC, HALO, T), BF16)

    qscale = DH ** -0.5 * math.log2(math.e)
    zero = zero_ref[0]

    def unpack_wq(pair, part):
        g, p = divmod(pair, H // 4)
        lo, hi = _split_heads(wq_raw[g, pl.ds(part * T * (H // 4) + p, T, stride=H // 4), :])
        w_v[zero + 2 * pair, part * T:(part + 1) * T, :] = lo
        w_v[zero + 2 * pair + 1, part * T:(part + 1) * T, :] = hi

    def unpack_wkv(ct, pair):
        k_rows, v_rows = aligned(DM // wr + ct, wr), aligned((DM + DC) // wr + ct, wr)
        g, p = divmod(pair, H // 4)
        k0, k1 = _split_heads(wuk_raw[ct, g, pl.ds(p, wr, stride=H // 4), :])
        v0, v1 = _split_heads(wuv_raw[ct, g, pl.ds(p, wr, stride=H // 4), :])
        w_v[2 * pair, k_rows, :] = k0
        w_v[2 * pair + 1, k_rows, :] = k1
        w_v[2 * pair, v_rows, :] = v0
        w_v[2 * pair + 1, v_rows, :] = v1

    def q_proj(h, r, n):
        rows = aligned(r, n)
        q_v[h, rows, :] = (_dot(aq_v[rows, :], w_v[h, :DM, :]) * qscale).astype(BF16)

    def k_proj(h, r):
        rows = slice(r * PM, (r + 1) * PM)
        k_v[rows, :] = _dot(c_v[rows, :], w_v[h, DM:DM + DC, :]).astype(BF16)

    def v_proj(h, r):
        rows = slice(r * PM, (r + 1) * PM)
        v_v[rows, :] = _dot(c_v[rows, :], w_v[h, DM + DC:, :]).astype(BF16)

    def conv_input(ct, i):
        sh = shift_ref[:, aligned(ct, T)].astype(F32)
        kf = ak_v[ct, i * T:(i + 1) * T + HALO, :].astype(F32)
        ksh = kf * sh[0:1, :]
        for j in range(1, KS):
            ksh = ksh + pltpu.roll(kf, j, 0) * sh[j:j + 1, :]
        rows = slice(i * T, (i + 1) * T)
        kv_v[rows, :] = (ksh[HALO:] * av_v[ct, rows, :].astype(F32)).astype(BF16)

    def input_spectrum(i):
        xf = _dot(fwd_ref[...], kv_v[i * T:(i + 1) * T, :])
        spec_v[XS + i] = xf[:T] + xf[T:]
        spec_v[XS + NB + i] = xf[:T]
        spec_v[XS + 2 * NB + i] = xf[T:]

    def kernel_spectrum(ct, i, prev):
        half = T // 2
        hf = _dot_nt(fwd_ref[...], ssmk_v[ct, :, i * T:(i + 1) * T])
        gr, gi = hf[:T], hf[T:]
        if i:
            pr, pi = prev[0][:T], prev[0][T:]
            gr = jnp.concatenate([gr[:half] - pi[:half], gr[half:] + pi[half:]], axis=0)
            gi = jnp.concatenate([gi[:half] + pr[:half], gi[half:] - pr[half:]], axis=0)
        prev[0] = hf
        spec_v[GS + i] = gr
        spec_v[GS + NB + i] = gi

    def conv_bins(lo, hi, f):
        rows = slice(8 * f, 8 * f + 8)

        def part(n):
            outs = [None] * (hi - lo)
            for j in range(hi):
                g = spec_v[GS + j, rows, :]
                if n:
                    gi = spec_v[GS + NB + j, rows, :]
                    g = gi - g if n == 1 else gi + g
                for i in range(max(lo, j), hi):
                    t = spec_v[XS + n * NB + i - j, rows, :] * g
                    outs[i - lo] = t if j == 0 else outs[i - lo] + t
            return outs

        s1 = part(0)
        re = [a - b for a, b in zip(s1, part(2))]
        im = [a + b for a, b in zip(s1, part(1))]
        base = YS + (zero if f % 4 == 3 else 0)
        for i in range(lo, hi):
            spec_v[base + 2 * i, rows, :] = re[i - lo]
            spec_v[base + 2 * i + 1, rows, :] = im[i - lo]

    def conv_inverse(ct, i):
        d = ssmd_v[pl.ds(ct, 1), :]
        rows = slice(i * T, (i + 1) * T)
        yf = jnp.concatenate([spec_v[YS + 2 * i], spec_v[YS + 2 * i + 1]], axis=0)
        y = _dot(inv_ref[...], yf.astype(BF16))
        y_v[ct, rows, :] = (y + kv_v[rows, :].astype(F32) * d).astype(BF16)

    def conv_tile(ct, fillers, slots):
        P = functools.partial
        fillers = iter(fillers)
        prev = [None]
        take = lambda n: [next(fillers) for _ in range(n)]
        blocks = lambda r: range(4 * r, 4 * r + 4)
        for r in range(-1, 4):
            side = []
            if r < 3:
                side += [P(conv_input, ct, i) for i in blocks(r + 1)]
                for i in blocks(r + 1):
                    side += [P(input_spectrum, i), P(kernel_spectrum, ct, i, prev)]
            if r > 0:
                side += [P(conv_inverse, ct, i) for i in blocks(r - 1)]
            bins = [P(conv_bins, 4 * r, 4 * r + 4, f) for f in range(T // 8)] if r >= 0 else []
            unpack = [P(unpack_wkv, ct, pair) for pair in blocks(r)] if r >= 0 else []
            _interleave(take(slots[r + 1]), bins, side, unpack)
        _interleave([P(conv_inverse, ct, i) for i in blocks(3)], list(fillers))

    P = functools.partial
    after_x = ((x_copy(1), x_copy(2)),
               (x_copy(3), *small_copies),
               conv_copies(0) + wkv_copies(0))
    parts = range(DM // T)
    wq_copy(0).wait()
    for n in range(3):
        x_copy(n).wait()
        for cp in after_x[n]:
            cp.start()
        steps = []
        for h in range(8):
            if n == 0 and h % 2 == 0:
                steps += [P(unpack_wq, h // 2, part) for part in parts]
            steps += [P(q_proj, h, r, T) for r in range(X_EDGES[n] // T, X_EDGES[n + 1] // T)]
        _interleave(steps, [P(unpack_wq, pair, part)
                            for pair in ((), (4, 5), (6, 7))[n] for part in parts])
    x_copy(3).wait()
    for cp in small_copies:
        cp.wait()
    ssmd_v[...] = ssmd_ref[...].astype(F32)
    chunks, first = S // PM, 4
    per_tile = (H * chunks - 8 * first) // NC

    def q_step(ct, carry):
        for cp in conv_copies(ct) + wkv_copies(ct):
            cp.wait()

        @pl.when(ct + 1 < NC)
        def _():
            for cp in conv_copies(ct + 1) + wkv_copies(ct + 1):
                cp.start()

        @pl.when(ct == 0)
        def _():
            wq_copy(1).start()

        @pl.when(ct == 2)
        def _():
            wq_copy(1).wait()
            c_copy.start()
            _interleave([P(q_proj, h, r, T) for h in range(8) for r in (6, 7)],
                        [P(unpack_wq, pair, part) for pair in range(8, 16) for part in parts])

        def piece(n):
            p = per_tile * ct + n
            early = p < 8 * (chunks - first)
            h = jnp.where(early, p % 8, (p + 8 * first) // chunks)
            r = jnp.where(early, first + p // 8, p % chunks)
            q_proj(h, r, PM)

        conv_tile(ct, [P(piece, n) for n in range(per_tile)], (2, 4, 6, 7, 8))
        return carry

    lax.fori_loop(0, NC, q_step, 0)
    c_copy.wait()
    wo_copy.start()
    for r in range(S // PM):
        k_proj(0, r)
        v_proj(0, r)

    def attend(h, next_head):
        tri = (lax.broadcasted_iota(jnp.int32, (T, T), 1)
               <= lax.broadcasted_iota(jnp.int32, (T, T), 0))

        def scores(i, st):
            q = q_v[h, i * T:(i + 1) * T, :]
            tiles, mx = [], None
            for c0 in range(0, i + 1, QK_TILES):
                c1 = min(c0 + QK_TILES, i + 1)
                s = _dot_nt(q, k_v[c0 * T:c1 * T, :])
                for j in range(c0, c1):
                    t = s[:, (j - c0) * T:(j - c0 + 1) * T]
                    if j == i:
                        t = jnp.where(tri, t, -1e9)
                    tiles.append(t)
                    mx = t if mx is None else jnp.maximum(mx, t)
                if c1 == i + 1:
                    st["m"] = jnp.max(mx, axis=1, keepdims=True)
                    st["tiles"] = tiles
                yield

        def context(i, st):
            m, tiles = st["m"], st["tiles"]
            o = l = None
            for c0 in range(0, i + 1, PV_TILES):
                c1 = min(c0 + PV_TILES, i + 1)
                ps = [jnp.exp2(t - m) for t in tiles[c0:c1]]
                for p in ps:
                    l = p if l is None else l + p
                if c1 > 1:
                    ps[-1] = jnp.minimum(ps[-1], l)
                pc = jnp.concatenate(ps, axis=1).astype(BF16)
                oc = _dot(pc, v_v[c0 * T:c1 * T, :])
                o = oc if o is None else o + oc
                if c1 == i + 1:
                    l = jnp.sum(l, axis=1, keepdims=True)
                    r = pl.reciprocal(l, approx=True)
                    r = r * (2.0 - l * r)
                    q_v[h, i * T:(i + 1) * T, :] = (o * r).astype(BF16)
                yield

        prev = iter(())
        for i in range(NB - 1, -1, -1):
            st = {}
            cur = scores(i, st)
            for _ in prev:
                next(cur, None)
            _finish(cur)
            if next_head is not None:
                if i < S // PM:
                    k_proj(next_head, i)
                if i + 1 < S // PM:
                    v_proj(next_head, i + 1)
            prev = context(i, st)
        _finish(prev)
        if next_head is not None:
            v_proj(next_head, 0)

    def attend_step(n, carry):
        attend(2 * n, 2 * n + 1)
        attend(2 * n + 1, 2 * n + 2)
        return carry

    lax.fori_loop(0, H // 2 - 1, attend_step, 0)
    attend(H - 2, H - 1)
    attend(H - 1, None)

    wo_copy.wait()

    def out_copy(r):
        return pltpu.make_async_copy(
            o_v.at[r], out_hbm.at[pl.ds(r * RB, RB), :], out_sem.at[r])

    def out_proj(r, carry):
        rows = pl.ds(pl.multiple_of(r * RB, RB), RB)
        ctx = jnp.concatenate([q_v[n, rows, :] for n in range(H)], axis=1)
        b = _dot(ctx, wo_v[...])
        aq = aq_v[rows, :].astype(F32)
        gw = gw_ref[...].astype(F32)
        gw = jnp.concatenate([gw[n:n + 1, :] for n in range(NC)], axis=1)
        g = jax.nn.sigmoid(jnp.sum(aq * gw, axis=1, keepdims=True))
        y = jnp.concatenate([y_v[n, rows, :].astype(F32) for n in range(NC)], axis=1)
        o_v[r] = (g * (aq * y) + (1.0 - g) * b).astype(BF16)
        out_copy(r).start()
        return carry

    lax.fori_loop(0, S // RB, out_proj, 0)
    for r in range(S // RB):
        out_copy(r).wait()


@jax.jit
def pallas_gated_mix__ssm_conv_h3__compressed_kv_cla__prompt_kernel(
    A_q: jax.Array,
    A_k: jax.Array,
    A_v: jax.Array,
    A_shift_k: jax.Array,
    A_ssm_k: jax.Array,
    A_ssm_D: jax.Array,
    B_x: jax.Array,
    B_c_kv: jax.Array,
    B_w_q: jax.Array,
    B_w_uk: jax.Array,
    B_w_uv: jax.Array,
    B_w_o: jax.Array,
    gate_w: jax.Array,
):
    del B_x
    hbm = pl.BlockSpec(memory_space=pl.ANY)
    out = pl.pallas_call(
        _kernel,
        out_shape=jax.ShapeDtypeStruct((S, DM), BF16),
        in_specs=[hbm] * 15,
        out_specs=hbm,
        scratch_shapes=[
            pltpu.VMEM((S, DM), BF16),
            pltpu.VMEM((NC, S + HALO, T), BF16),
            pltpu.VMEM((NC, S, T), BF16),
            pltpu.VMEM((NC, T, S), BF16),
            pltpu.VMEM((S, DC), BF16),
            pltpu.VMEM((2, DM * H // 4, DH), U32),
            pltpu.VMEM((NC, 2, DC // NC * H // 4, DH), U32),
            pltpu.VMEM((NC, 2, DC // NC * H // 4, DH), U32),
            pltpu.VMEM((H * DH, DM), BF16),
            pltpu.VMEM((H, DM + 2 * DC, DH), BF16),
            pltpu.VMEM((H, S, DH), BF16),
            pltpu.VMEM((S, DH), BF16),
            pltpu.VMEM((S, DH), BF16),
            pltpu.VMEM((NC, S, T), BF16),
            pltpu.VMEM((S, T), BF16),
            pltpu.VMEM((7 * NB, T, T), F32),
            pltpu.VMEM((S // RB, RB, DM), BF16),
            pltpu.VMEM((2 * T, T), BF16),
            pltpu.VMEM((T, 2 * T), BF16),
            pltpu.VMEM((KS, DM), BF16),
            pltpu.VMEM((NC, T), BF16),
            pltpu.VMEM((NC, T), BF16),
            pltpu.VMEM((NC, T), F32),
            pltpu.SMEM((1,), jnp.int32),
            pltpu.SemaphoreType.DMA((5,)),
            pltpu.SemaphoreType.DMA((4,)),
            pltpu.SemaphoreType.DMA((2,)),
            pltpu.SemaphoreType.DMA((3 * NC,)),
            pltpu.SemaphoreType.DMA((4 * NC,)),
            pltpu.SemaphoreType.DMA((3,)),
            pltpu.SemaphoreType.DMA((S // RB,)),
        ],
        compiler_params=pltpu.CompilerParams(vmem_limit_bytes=126 * 2**20),
        name="gated_mix_h3_cla",
    )(
        A_q.reshape(S, DM), A_k.reshape(S, DM), A_v.reshape(S, DM), A_ssm_k,
        B_c_kv.reshape(S, DC), B_w_q, B_w_uk, B_w_uv, B_w_o.reshape(H * DH, DM),
        jnp.zeros((1,), jnp.int32), A_shift_k.T, A_ssm_D.reshape(NC, T), gate_w.reshape(NC, T),
        jnp.asarray(_FWD, BF16), jnp.asarray(_INV, BF16),
    )
    return out.reshape(1, S, DM)
```

```python
import functools
import math

import jax
import jax.numpy as jnp
import numpy as np
from jax import lax
import jax.experimental.pallas as pl
import jax.experimental.pallas.tpu as pltpu

F32 = jnp.float32
BF16 = jnp.bfloat16
U32 = jnp.uint32

S = 2048
DM = 1024
H = 32
DH = 128
DC = 512
KS = 4
T = 128
NB = S // T
NC = DM // T
PM = 256
RB = 256
QK_TILES = 4
PV_TILES = 2
X_EDGES = (0, 128, 384, 768, S)
XS, GS, YS = 0, 3 * NB, 5 * NB
HALO = 16


def _dft_matrices():
    even = np.arange(0, T, 2)
    k = np.concatenate([even, T - 1 - even]).astype(np.float64)
    ang = 2.0 * np.pi * np.outer(k + 0.5, np.arange(T)) / (2 * T)
    fwd = np.concatenate([np.cos(ang), -np.sin(ang)], axis=0)
    inv = np.concatenate([np.cos(ang[:T // 2]), -np.sin(ang[:T // 2])], axis=0).T / T
    inv = np.concatenate([inv[0::2], inv[1::2]], axis=0)
    return fwd.astype(np.float32), inv.astype(np.float32)


_FWD, _INV = _dft_matrices()


def _dot(a, b):
    return jnp.dot(a, b, preferred_element_type=F32)


def _dot_nt(a, b):
    return lax.dot_general(a, b, (((1,), (1,)), ((), ())), preferred_element_type=F32)


def _unpack(w):
    return (lax.bitcast_convert_type(w << 16, F32),
            lax.bitcast_convert_type(w & jnp.uint32(0xFFFF0000), F32))


def _split_heads(w):
    lo, hi = _unpack(w)
    return lo.astype(BF16), hi.astype(BF16)


def _finish(gen):
    for _ in gen:
        pass


def _interleave(*streams):
    steps = [((n + 0.5 * (k > 0)) / len(st), k, fn)
             for k, st in enumerate(streams) for n, fn in enumerate(st)]
    for _, _, fn in sorted(steps, key=lambda t: t[:2]):
        fn()


def _kernel(
    aq_hbm, ak_hbm, av_hbm, ssmk_hbm, c_hbm, wq_hbm, wuk_hbm, wuv_hbm, wo_hbm,
    zero_hbm, shift_hbm, ssmd_hbm, gw_hbm, fwd_hbm, inv_hbm,
    out_hbm,
    aq_v, ak_v, av_v, ssmk_v, c_v, wq_raw, wuk_raw, wuv_raw, wo_v,
    w_v, q_v, k_v, v_v, y_v, kv_v, spec_v, o_v,
    fwd_ref, inv_ref, shift_ref, ssmd_ref, gw_ref, ssmd_v, zero_ref,
    small_sem, x_sem, wq_sem, conv_sem, wkv_sem, misc_sem, out_sem,
):
    wr = DC // NC

    def aligned(i, n):
        return pl.ds(i * n if isinstance(i, int) else pl.multiple_of(i * n, n), n)

    def x_copy(n):
        rows = pl.ds(X_EDGES[n], X_EDGES[n + 1] - X_EDGES[n])
        return pltpu.make_async_copy(aq_hbm.at[rows], aq_v.at[rows], x_sem.at[n])

    def wq_copy(g):
        pairs = H // 4
        return pltpu.make_async_copy(
            wq_hbm.bitcast(U32).at[:, pl.ds(g * pairs, pairs), :],
            wq_raw.at[g].reshape(DM, pairs, DH), wq_sem.at[g])

    def conv_copies(ct):
        ch = aligned(ct, T)
        return (
            pltpu.make_async_copy(ak_hbm.at[:, ch], ak_v.at[ct, pl.ds(HALO, S)], conv_sem.at[3 * ct]),
            pltpu.make_async_copy(av_hbm.at[:, ch], av_v.at[ct], conv_sem.at[3 * ct + 1]),
            pltpu.make_async_copy(ssmk_hbm.at[ch], ssmk_v.at[ct], conv_sem.at[3 * ct + 2]),
        )

    def wkv_copies(ct):
        pairs = H // 4
        return tuple(
            pltpu.make_async_copy(
                src.bitcast(U32).at[aligned(ct, wr), pl.ds(g * pairs, pairs), :],
                dst.at[ct, g].reshape(wr, pairs, DH), wkv_sem.at[4 * ct + 2 * n + g])
            for n, (src, dst) in enumerate(((wuk_hbm, wuk_raw), (wuv_hbm, wuv_raw)))
            for g in range(2))

    c_copy = pltpu.make_async_copy(c_hbm, c_v, misc_sem.at[0])
    wo_copy = pltpu.make_async_copy(wo_hbm, wo_v, misc_sem.at[1])

    small_copies = [
        pltpu.make_async_copy(src, dst, small_sem.at[n]) for n, (src, dst) in enumerate((
            (shift_hbm, shift_ref), (ssmd_hbm, ssmd_ref), (gw_hbm, gw_ref),
            (fwd_hbm, fwd_ref), (inv_hbm, inv_ref)))]
    zero_copy = pltpu.make_async_copy(zero_hbm, zero_ref, misc_sem.at[2])

    zero_copy.start()
    wq_copy(0).start()
    x_copy(0).start()
    zero_copy.wait()

    ak_v[:, 0:HALO, :] = jnp.zeros((NC, HALO, T), BF16)

    qscale = DH ** -0.5 * math.log2(math.e)
    zero = zero_ref[0]

    def unpack_wq(pair, part):
        g, p = divmod(pair, H // 4)
        lo, hi = _split_heads(wq_raw[g, pl.ds(part * T * (H // 4) + p, T, stride=H // 4), :])
        w_v[zero + 2 * pair, part * T:(part + 1) * T, :] = lo
        w_v[zero + 2 * pair + 1, part * T:(part + 1) * T, :] = hi

    def unpack_wkv(ct, pair):
        k_rows, v_rows = aligned(DM // wr + ct, wr), aligned((DM + DC) // wr + ct, wr)
        g, p = divmod(pair, H // 4)
        k0, k1 = _split_heads(wuk_raw[ct, g, pl.ds(p, wr, stride=H // 4), :])
        v0, v1 = _split_heads(wuv_raw[ct, g, pl.ds(p, wr, stride=H // 4), :])
        w_v[2 * pair, k_rows, :] = k0
        w_v[2 * pair + 1, k_rows, :] = k1
        w_v[2 * pair, v_rows, :] = v0
        w_v[2 * pair + 1, v_rows, :] = v1

    def q_proj(h, r, n):
        rows = aligned(r, n)
        q_v[h, rows, :] = (_dot(aq_v[rows, :], w_v[h, :DM, :]) * qscale).astype(BF16)

    def k_proj(h, r):
        rows = slice(r * PM, (r + 1) * PM)
        k_v[rows, :] = _dot(c_v[rows, :], w_v[h, DM:DM + DC, :]).astype(BF16)

    def v_proj(h, r):
        rows = slice(r * PM, (r + 1) * PM)
        v_v[rows, :] = _dot(c_v[rows, :], w_v[h, DM + DC:, :]).astype(BF16)

    def conv_input(ct, i):
        sh = shift_ref[:, aligned(ct, T)].astype(F32)
        kf = ak_v[ct, i * T:(i + 1) * T + HALO, :].astype(F32)
        ksh = kf * sh[0:1, :]
        for j in range(1, KS):
            ksh = ksh + pltpu.roll(kf, j, 0) * sh[j:j + 1, :]
        rows = slice(i * T, (i + 1) * T)
        kv_v[rows, :] = (ksh[HALO:] * av_v[ct, rows, :].astype(F32)).astype(BF16)

    def input_spectrum(i):
        xf = _dot(fwd_ref[...], kv_v[i * T:(i + 1) * T, :])
        spec_v[XS + i] = xf[:T] + xf[T:]
        spec_v[XS + NB + i] = xf[:T]
        spec_v[XS + 2 * NB + i] = xf[T:]

    def kernel_spectrum(ct, i, prev):
        half = T // 2
        hf = _dot_nt(fwd_ref[...], ssmk_v[ct, :, i * T:(i + 1) * T])
        gr, gi = hf[:T], hf[T:]
        if i:
            pr, pi = prev[0][:T], prev[0][T:]
            gr = jnp.concatenate([gr[:half] - pi[:half], gr[half:] + pi[half:]], axis=0)
            gi = jnp.concatenate([gi[:half] + pr[:half], gi[half:] - pr[half:]], axis=0)
        prev[0] = hf
        spec_v[GS + i] = gr
        spec_v[GS + NB + i] = gi

    def conv_bins(lo, hi, f):
        rows = slice(8 * f, 8 * f + 8)

        def part(n):
            outs = [None] * (hi - lo)
            for j in range(hi):
                g = spec_v[GS + j, rows, :]
                if n:
                    gi = spec_v[GS + NB + j, rows, :]
                    g = gi - g if n == 1 else gi + g
                for i in range(max(lo, j), hi):
                    t = spec_v[XS + n * NB + i - j, rows, :] * g
                    outs[i - lo] = t if j == 0 else outs[i - lo] + t
            return outs

        s1 = part(0)
        re = [a - b for a, b in zip(s1, part(2))]
        im = [a + b for a, b in zip(s1, part(1))]
        base = YS + (zero if f % 4 == 3 else 0)
        for i in range(lo, hi):
            spec_v[base + 2 * i, rows, :] = re[i - lo]
            spec_v[base + 2 * i + 1, rows, :] = im[i - lo]

    def conv_inverse(ct, i):
        d = ssmd_v[pl.ds(ct, 1), :]
        half = T // 2
        re, im = spec_v[YS + 2 * i], spec_v[YS + 2 * i + 1]
        folded = (jnp.concatenate([re[:half] + re[half:], im[:half] - im[half:]], axis=0),
                  jnp.concatenate([re[:half] - re[half:], im[:half] + im[half:]], axis=0))
        kv = _unpack(pltpu.bitcast(kv_v[i * T:(i + 1) * T, :], U32))
        for odd in range(2):
            y = _dot(inv_ref[odd * half:(odd + 1) * half, :], folded[odd].astype(BF16))
            y_v[ct, pl.ds(i * T + odd, half, stride=2), :] = y + kv[odd] * d

    def conv_tile(ct, fillers, slots):
        P = functools.partial
        fillers = iter(fillers)
        prev = [None]
        take = lambda n: [next(fillers) for _ in range(n)]
        blocks = lambda r: range(4 * r, 4 * r + 4)
        for r in range(-1, 4):
            side = []
            if r < 3:
                side += [P(conv_input, ct, i) for i in blocks(r + 1)]
                for i in blocks(r + 1):
                    side += [P(input_spectrum, i), P(kernel_spectrum, ct, i, prev)]
            if r > 0:
                side += [P(conv_inverse, ct, i) for i in blocks(r - 1)]
            bins = [P(conv_bins, 4 * r, 4 * r + 4, f) for f in range(T // 8)] if r >= 0 else []
            unpack = [P(unpack_wkv, ct, pair) for pair in blocks(r)] if r >= 0 else []
            _interleave(take(slots[r + 1]), bins, side, unpack)
        _interleave([P(conv_inverse, ct, i) for i in blocks(3)], list(fillers))

    P = functools.partial
    after_x = ((x_copy(1), x_copy(2)),
               (x_copy(3), *small_copies),
               conv_copies(0) + wkv_copies(0))
    parts = range(DM // T)
    wq_copy(0).wait()
    for n in range(3):
        x_copy(n).wait()
        for cp in after_x[n]:
            cp.start()
        steps = []
        for h in range(8):
            if n == 0 and h % 2 == 0:
                steps += [P(unpack_wq, h // 2, part) for part in parts]
            steps += [P(q_proj, h, r, T) for r in range(X_EDGES[n] // T, X_EDGES[n + 1] // T)]
        _interleave(steps, [P(unpack_wq, pair, part)
                            for pair in ((), (4, 5), (6, 7))[n] for part in parts])
    x_copy(3).wait()
    for cp in small_copies:
        cp.wait()
    ssmd_v[...] = ssmd_ref[...].astype(F32)
    chunks, first = S // PM, 4
    per_tile = (H * chunks - 8 * first) // NC

    def q_step(ct, carry):
        for cp in conv_copies(ct) + wkv_copies(ct):
            cp.wait()

        @pl.when(ct + 1 < NC)
        def _():
            for cp in conv_copies(ct + 1) + wkv_copies(ct + 1):
                cp.start()

        @pl.when(ct == 0)
        def _():
            wq_copy(1).start()

        @pl.when(ct == 2)
        def _():
            wq_copy(1).wait()
            c_copy.start()
            _interleave([P(q_proj, h, r, T) for h in range(8) for r in (6, 7)],
                        [P(unpack_wq, pair, part) for pair in range(8, 16) for part in parts])

        def piece(n):
            p = per_tile * ct + n
            early = p < 8 * (chunks - first)
            h = jnp.where(early, p % 8, (p + 8 * first) // chunks)
            r = jnp.where(early, first + p // 8, p % chunks)
            q_proj(h, r, PM)

        conv_tile(ct, [P(piece, n) for n in range(per_tile)], (2, 4, 6, 7, 8))
        return carry

    lax.fori_loop(0, NC, q_step, 0)
    c_copy.wait()
    wo_copy.start()
    for r in range(S // PM):
        k_proj(0, r)
        v_proj(0, r)

    def attend(h, next_head):
        tri = (lax.broadcasted_iota(jnp.int32, (T, T), 1)
               <= lax.broadcasted_iota(jnp.int32, (T, T), 0))

        def scores(i, st):
            q = q_v[h, i * T:(i + 1) * T, :]
            tiles, mx = [], None
            for c0 in range(0, i + 1, QK_TILES):
                c1 = min(c0 + QK_TILES, i + 1)
                s = _dot_nt(q, k_v[c0 * T:c1 * T, :])
                for j in range(c0, c1):
                    t = s[:, (j - c0) * T:(j - c0 + 1) * T]
                    if j == i:
                        t = jnp.where(tri, t, -1e9)
                    tiles.append(t)
                    mx = t if mx is None else jnp.maximum(mx, t)
                if c1 == i + 1:
                    st["m"] = jnp.max(mx, axis=1, keepdims=True)
                    st["tiles"] = tiles
                yield

        def context(i, st):
            m, tiles = st["m"], st["tiles"]
            o = l = None
            for c0 in range(0, i + 1, PV_TILES):
                c1 = min(c0 + PV_TILES, i + 1)
                ps = [jnp.exp2(t - m) for t in tiles[c0:c1]]
                for p in ps:
                    l = p if l is None else l + p
                if c1 > 1:
                    ps[-1] = jnp.minimum(ps[-1], l)
                pc = jnp.concatenate(ps, axis=1).astype(BF16)
                oc = _dot(pc, v_v[c0 * T:c1 * T, :])
                o = oc if o is None else o + oc
                if c1 == i + 1:
                    l = jnp.sum(l, axis=1, keepdims=True)
                    r = pl.reciprocal(l, approx=True)
                    r = r * (2.0 - l * r)
                    q_v[h, i * T:(i + 1) * T, :] = (o * r).astype(BF16)
                yield

        prev = iter(())
        for i in range(NB - 1, -1, -1):
            st = {}
            cur = scores(i, st)
            for _ in prev:
                next(cur, None)
            _finish(cur)
            if next_head is not None:
                if i < S // PM:
                    k_proj(next_head, i)
                if i + 1 < S // PM:
                    v_proj(next_head, i + 1)
            prev = context(i, st)
        _finish(prev)
        if next_head is not None:
            v_proj(next_head, 0)

    def attend_step(n, carry):
        attend(2 * n, 2 * n + 1)
        attend(2 * n + 1, 2 * n + 2)
        return carry

    lax.fori_loop(0, H // 2 - 1, attend_step, 0)
    attend(H - 2, H - 1)
    attend(H - 1, None)

    wo_copy.wait()

    def out_copy(r):
        return pltpu.make_async_copy(
            o_v.at[r], out_hbm.at[pl.ds(r * RB, RB), :], out_sem.at[r])

    def out_proj(r, carry):
        rows = pl.ds(pl.multiple_of(r * RB, RB), RB)
        ctx = jnp.concatenate([q_v[n, rows, :] for n in range(H)], axis=1)
        b = _dot(ctx, wo_v[...])
        aq = aq_v[rows, :].astype(F32)
        gw = gw_ref[...].astype(F32)
        gw = jnp.concatenate([gw[n:n + 1, :] for n in range(NC)], axis=1)
        g = jax.nn.sigmoid(jnp.sum(aq * gw, axis=1, keepdims=True))
        y = jnp.concatenate([y_v[n, rows, :] for n in range(NC)], axis=1)
        o_v[r] = (g * (aq * y) + (1.0 - g) * b).astype(BF16)
        out_copy(r).start()
        return carry

    lax.fori_loop(0, S // RB, out_proj, 0)
    for r in range(S // RB):
        out_copy(r).wait()


@jax.jit
def pallas_gated_mix__ssm_conv_h3__compressed_kv_cla__prompt_kernel(
    A_q: jax.Array,
    A_k: jax.Array,
    A_v: jax.Array,
    A_shift_k: jax.Array,
    A_ssm_k: jax.Array,
    A_ssm_D: jax.Array,
    B_x: jax.Array,
    B_c_kv: jax.Array,
    B_w_q: jax.Array,
    B_w_uk: jax.Array,
    B_w_uv: jax.Array,
    B_w_o: jax.Array,
    gate_w: jax.Array,
):
    del B_x
    hbm = pl.BlockSpec(memory_space=pl.ANY)
    out = pl.pallas_call(
        _kernel,
        out_shape=jax.ShapeDtypeStruct((S, DM), BF16),
        in_specs=[hbm] * 15,
        out_specs=hbm,
        scratch_shapes=[
            pltpu.VMEM((S, DM), BF16),
            pltpu.VMEM((NC, S + HALO, T), BF16),
            pltpu.VMEM((NC, S, T), BF16),
            pltpu.VMEM((NC, T, S), BF16),
            pltpu.VMEM((S, DC), BF16),
            pltpu.VMEM((2, DM * H // 4, DH), U32),
            pltpu.VMEM((NC, 2, DC // NC * H // 4, DH), U32),
            pltpu.VMEM((NC, 2, DC // NC * H // 4, DH), U32),
            pltpu.VMEM((H * DH, DM), BF16),
            pltpu.VMEM((H, DM + 2 * DC, DH), BF16),
            pltpu.VMEM((H, S, DH), BF16),
            pltpu.VMEM((S, DH), BF16),
            pltpu.VMEM((S, DH), BF16),
            pltpu.VMEM((NC, S, T), F32),
            pltpu.VMEM((S, T), BF16),
            pltpu.VMEM((7 * NB, T, T), F32),
            pltpu.VMEM((S // RB, RB, DM), BF16),
            pltpu.VMEM((2 * T, T), BF16),
            pltpu.VMEM((T, T), BF16),
            pltpu.VMEM((KS, DM), BF16),
            pltpu.VMEM((NC, T), BF16),
            pltpu.VMEM((NC, T), BF16),
            pltpu.VMEM((NC, T), F32),
            pltpu.SMEM((1,), jnp.int32),
            pltpu.SemaphoreType.DMA((5,)),
            pltpu.SemaphoreType.DMA((4,)),
            pltpu.SemaphoreType.DMA((2,)),
            pltpu.SemaphoreType.DMA((3 * NC,)),
            pltpu.SemaphoreType.DMA((4 * NC,)),
            pltpu.SemaphoreType.DMA((3,)),
            pltpu.SemaphoreType.DMA((S // RB,)),
        ],
        compiler_params=pltpu.CompilerParams(vmem_limit_bytes=126 * 2**20),
        name="gated_mix_h3_cla",
    )(
        A_q.reshape(S, DM), A_k.reshape(S, DM), A_v.reshape(S, DM), A_ssm_k,
        B_c_kv.reshape(S, DC), B_w_q, B_w_uk, B_w_uv, B_w_o.reshape(H * DH, DM),
        jnp.zeros((1,), jnp.int32), A_shift_k.T, A_ssm_D.reshape(NC, T), gate_w.reshape(NC, T),
        jnp.asarray(_FWD, BF16), jnp.asarray(_INV, BF16),
    )
    return out.reshape(1, S, DM)
```

```python
import functools
import math

import jax
import jax.numpy as jnp
import numpy as np
from jax import lax
import jax.experimental.pallas as pl
import jax.experimental.pallas.tpu as pltpu

F32 = jnp.float32
BF16 = jnp.bfloat16
U32 = jnp.uint32

S = 2048
DM = 1024
H = 32
DH = 128
DC = 512
KS = 4
T = 128
NB = S // T
NC = DM // T
PM = 256
RB = 256
QK_TILES = 4
PV_TILES = 2
X_EDGES = (0, 128, 384, 768, S)
XS, GS, YS = 0, 3 * NB, 5 * NB
HALO = 16


def _dft_matrices():
    even = np.arange(0, T, 2)
    k = np.concatenate([even, T - 1 - even]).astype(np.float64)
    ang = 2.0 * np.pi * np.outer(k + 0.5, np.arange(T)) / (2 * T)
    fwd = np.concatenate([np.cos(ang), -np.sin(ang)], axis=0)
    inv = np.concatenate([np.cos(ang[:T // 2]), -np.sin(ang[:T // 2])], axis=0).T / T
    inv = np.concatenate([inv[0::2], inv[1::2]], axis=0)
    return fwd.astype(np.float32), inv.astype(np.float32)


_FWD, _INV = _dft_matrices()


def _dot(a, b):
    return jnp.dot(a, b, preferred_element_type=F32)


def _dot_nt(a, b):
    return lax.dot_general(a, b, (((1,), (1,)), ((), ())), preferred_element_type=F32)


def _unpack(w):
    return (lax.bitcast_convert_type(w << 16, F32),
            lax.bitcast_convert_type(w & jnp.uint32(0xFFFF0000), F32))


def _split_heads(w):
    lo, hi = _unpack(w)
    return lo.astype(BF16), hi.astype(BF16)


def _finish(gen):
    for _ in gen:
        pass


def _interleave(*streams):
    steps = [((n + 0.5 * (k > 0)) / len(st), k, fn)
             for k, st in enumerate(streams) for n, fn in enumerate(st)]
    for _, _, fn in sorted(steps, key=lambda t: t[:2]):
        fn()


def _kernel(
    aq_hbm, ak_hbm, av_hbm, ssmk_hbm, c_hbm, wq_hbm, wuk_hbm, wuv_hbm, wo_hbm,
    zero_hbm, shift_hbm, ssmd_hbm, gw_hbm, fwd_hbm, inv_hbm,
    out_hbm,
    aq_v, ak_v, av_v, ssmk_v, c_v, wq_raw, wuk_raw, wuv_raw, wo_v,
    w_v, q_v, k_v, v_v, y_v, kv_v, spec_v, o_v,
    fwd_ref, inv_ref, shift_ref, ssmd_ref, gw_ref, ssmd_v, zero_ref,
    small_sem, x_sem, wq_sem, conv_sem, wkv_sem, misc_sem, out_sem,
):
    wr = DC // NC

    def aligned(i, n):
        return pl.ds(i * n if isinstance(i, int) else pl.multiple_of(i * n, n), n)

    def x_copy(n):
        rows = pl.ds(X_EDGES[n], X_EDGES[n + 1] - X_EDGES[n])
        return pltpu.make_async_copy(aq_hbm.at[rows], aq_v.at[rows], x_sem.at[n])

    def wq_copy(g):
        pairs = H // 4
        return pltpu.make_async_copy(
            wq_hbm.bitcast(U32).at[:, pl.ds(g * pairs, pairs), :],
            wq_raw.at[g].reshape(DM, pairs, DH), wq_sem.at[g])

    def conv_copies(ct):
        ch = aligned(ct, T)
        return (
            pltpu.make_async_copy(ak_hbm.at[:, ch], ak_v.at[ct, pl.ds(HALO, S)], conv_sem.at[3 * ct]),
            pltpu.make_async_copy(av_hbm.at[:, ch], av_v.at[ct], conv_sem.at[3 * ct + 1]),
            pltpu.make_async_copy(ssmk_hbm.at[ch], ssmk_v.at[ct], conv_sem.at[3 * ct + 2]),
        )

    def wkv_copies(ct):
        pairs = H // 4
        return tuple(
            pltpu.make_async_copy(
                src.bitcast(U32).at[aligned(ct, wr), pl.ds(g * pairs, pairs), :],
                dst.at[ct, g].reshape(wr, pairs, DH), wkv_sem.at[4 * ct + 2 * n + g])
            for n, (src, dst) in enumerate(((wuk_hbm, wuk_raw), (wuv_hbm, wuv_raw)))
            for g in range(2))

    c_copy = pltpu.make_async_copy(c_hbm, c_v, misc_sem.at[0])
    wo_copy = pltpu.make_async_copy(wo_hbm, wo_v, misc_sem.at[1])

    small_copies = [
        pltpu.make_async_copy(src, dst, small_sem.at[n]) for n, (src, dst) in enumerate((
            (shift_hbm, shift_ref), (ssmd_hbm, ssmd_ref), (gw_hbm, gw_ref),
            (fwd_hbm, fwd_ref), (inv_hbm, inv_ref)))]
    zero_copy = pltpu.make_async_copy(zero_hbm, zero_ref, misc_sem.at[2])

    zero_copy.start()
    wq_copy(0).start()
    x_copy(0).start()
    zero_copy.wait()

    ak_v[:, 0:HALO, :] = jnp.zeros((NC, HALO, T), BF16)

    qscale = DH ** -0.5 * math.log2(math.e)
    zero = zero_ref[0]

    def unpack_wq(pair, part):
        g, p = divmod(pair, H // 4)
        lo, hi = _split_heads(wq_raw[g, pl.ds(part * T * (H // 4) + p, T, stride=H // 4), :])
        w_v[zero + 2 * pair, part * T:(part + 1) * T, :] = lo
        w_v[zero + 2 * pair + 1, part * T:(part + 1) * T, :] = hi

    def unpack_wkv(ct, pair):
        k_rows, v_rows = aligned(DM // wr + ct, wr), aligned((DM + DC) // wr + ct, wr)
        g, p = divmod(pair, H // 4)
        k0, k1 = _split_heads(wuk_raw[ct, g, pl.ds(p, wr, stride=H // 4), :])
        v0, v1 = _split_heads(wuv_raw[ct, g, pl.ds(p, wr, stride=H // 4), :])
        w_v[2 * pair, k_rows, :] = k0
        w_v[2 * pair + 1, k_rows, :] = k1
        w_v[2 * pair, v_rows, :] = v0
        w_v[2 * pair + 1, v_rows, :] = v1

    def q_proj(h, r, n):
        rows = aligned(r, n)
        q_v[h, rows, :] = (_dot(aq_v[rows, :], w_v[h, :DM, :]) * qscale).astype(BF16)

    def k_proj(h, r):
        rows = slice(r * PM, (r + 1) * PM)
        k_v[rows, :] = _dot(c_v[rows, :], w_v[h, DM:DM + DC, :]).astype(BF16)

    def v_proj(h, r):
        rows = slice(r * PM, (r + 1) * PM)
        v_v[rows, :] = _dot(c_v[rows, :], w_v[h, DM + DC:, :]).astype(BF16)

    def conv_input(ct, i):
        sh = shift_ref[:, aligned(ct, T)].astype(F32)
        kf = ak_v[ct, i * T:(i + 1) * T + HALO, :].astype(F32)
        ksh = kf * sh[0:1, :]
        for j in range(1, KS):
            ksh = ksh + pltpu.roll(kf, j, 0) * sh[j:j + 1, :]
        rows = slice(i * T, (i + 1) * T)
        kv_v[rows, :] = (ksh[HALO:] * av_v[ct, rows, :].astype(F32)).astype(BF16)

    def input_spectrum(i):
        xf = _dot(fwd_ref[...], kv_v[i * T:(i + 1) * T, :])
        spec_v[XS + i] = xf[:T] + xf[T:]
        spec_v[XS + NB + i] = xf[:T]
        spec_v[XS + 2 * NB + i] = xf[T:]

    def kernel_spectrum(ct, i, prev):
        half = T // 2
        hf = _dot_nt(fwd_ref[...], ssmk_v[ct, :, i * T:(i + 1) * T])
        gr, gi = hf[:T], hf[T:]
        if i:
            pr, pi = prev[0][:T], prev[0][T:]
            gr = jnp.concatenate([gr[:half] - pi[:half], gr[half:] + pi[half:]], axis=0)
            gi = jnp.concatenate([gi[:half] + pr[:half], gi[half:] - pr[half:]], axis=0)
        prev[0] = hf
        spec_v[GS + i] = gr
        spec_v[GS + NB + i] = gi

    def conv_bins(lo, hi, f):
        rows = slice(8 * f, 8 * f + 8)

        def part(n):
            outs = [None] * (hi - lo)
            for j in range(hi):
                g = spec_v[GS + j, rows, :]
                if n:
                    gi = spec_v[GS + NB + j, rows, :]
                    g = gi - g if n == 1 else gi + g
                for i in range(max(lo, j), hi):
                    t = spec_v[XS + n * NB + i - j, rows, :] * g
                    outs[i - lo] = t if j == 0 else outs[i - lo] + t
            return outs

        s1 = part(0)
        re = [a - b for a, b in zip(s1, part(2))]
        im = [a + b for a, b in zip(s1, part(1))]
        base = YS + (zero if f % 4 == 3 else 0)
        for i in range(lo, hi):
            spec_v[base + 2 * i, rows, :] = re[i - lo]
            spec_v[base + 2 * i + 1, rows, :] = im[i - lo]

    def conv_inverse(ct, i):
        d = ssmd_v[pl.ds(ct, 1), :]
        half = T // 2
        re, im = spec_v[YS + 2 * i], spec_v[YS + 2 * i + 1]
        folded = (jnp.concatenate([re[:half] + re[half:], im[:half] - im[half:]], axis=0),
                  jnp.concatenate([re[:half] - re[half:], im[:half] + im[half:]], axis=0))
        kv = _unpack(pltpu.bitcast(kv_v[i * T:(i + 1) * T, :], U32))
        for odd in range(2):
            y = _dot(inv_ref[odd * half:(odd + 1) * half, :], folded[odd].astype(BF16))
            y_v[ct, pl.ds(i * T + odd, half, stride=2), :] = y + kv[odd] * d

    def conv_tile(ct, fillers):
        P = functools.partial
        slots = (0, 2, 6, 12, 19, len(fillers))
        inputs = (0, 6, 12, NB, NB, NB)
        prev = [None]
        for r in range(-1, 4):
            new = range(inputs[r + 1], inputs[r + 2])
            side = [P(conv_input, ct, i) for i in new]
            for i in new:
                side.append(P(input_spectrum, i))
                if r < 0:
                    side += [P(kernel_spectrum, ct, j, prev)
                             for j in range(i * NB // len(new), (i + 1) * NB // len(new))]
            if r > 0:
                side += [P(conv_inverse, ct, i) for i in range(4 * r - 4, 4 * r)]
            bins, unpack = [], []
            if r >= 0:
                bins = [P(conv_bins, 4 * r, 4 * r + 4, f) for f in range(T // 8)]
                unpack = [P(unpack_wkv, ct, pair) for pair in range(4 * r, 4 * r + 4)]
            _interleave(fillers[slots[r + 1]:slots[r + 2]], bins, side, unpack)
        for i in range(NB - 4, NB):
            conv_inverse(ct, i)

    P = functools.partial
    after_x = ((x_copy(1), x_copy(2)),
               (x_copy(3), *small_copies),
               conv_copies(0) + wkv_copies(0))
    parts = range(DM // T)
    wq_copy(0).wait()
    for n in range(3):
        x_copy(n).wait()
        for cp in after_x[n]:
            cp.start()
        steps = []
        for h in range(8):
            if n == 0 and h % 2 == 0:
                steps += [P(unpack_wq, h // 2, part) for part in parts]
            steps += [P(q_proj, h, r, T) for r in range(X_EDGES[n] // T, X_EDGES[n + 1] // T)]
        _interleave(steps, [P(unpack_wq, pair, part)
                            for pair in ((), (4, 5), (6, 7))[n] for part in parts])
    x_copy(3).wait()
    for cp in small_copies:
        cp.wait()
    ssmd_v[...] = ssmd_ref[...].astype(F32)
    chunks, first = S // PM, 4
    per_tile = (H * chunks - 8 * first) // NC

    def q_step(ct, carry):
        for cp in conv_copies(ct) + wkv_copies(ct):
            cp.wait()

        @pl.when(ct + 1 < NC)
        def _():
            for cp in conv_copies(ct + 1) + wkv_copies(ct + 1):
                cp.start()

        @pl.when(ct == 0)
        def _():
            wq_copy(1).start()

        @pl.when(ct == 2)
        def _():
            wq_copy(1).wait()
            c_copy.start()
            _interleave([P(q_proj, h, r, T) for h in range(8) for r in (6, 7)],
                        [P(unpack_wq, pair, part) for pair in range(8, 16) for part in parts])

        def piece(n):
            p = per_tile * ct + n
            early = p < 8 * (chunks - first)
            h = jnp.where(early, p % 8, (p + 8 * first) // chunks)
            r = jnp.where(early, first + p // 8, p % chunks)
            q_proj(h, r, PM)

        conv_tile(ct, [P(piece, n) for n in range(per_tile)])
        return carry

    lax.fori_loop(0, NC, q_step, 0)
    c_copy.wait()
    wo_copy.start()
    for r in range(S // PM):
        k_proj(0, r)
        v_proj(0, r)

    def attend(h, next_head):
        tri = (lax.broadcasted_iota(jnp.int32, (T, T), 1)
               <= lax.broadcasted_iota(jnp.int32, (T, T), 0))

        def scores(i, st):
            q = q_v[h, i * T:(i + 1) * T, :]
            tiles, mx = [], None
            for c0 in range(0, i + 1, QK_TILES):
                c1 = min(c0 + QK_TILES, i + 1)
                s = _dot_nt(q, k_v[c0 * T:c1 * T, :])
                for j in range(c0, c1):
                    t = s[:, (j - c0) * T:(j - c0 + 1) * T]
                    if j == i:
                        t = jnp.where(tri, t, -1e9)
                    tiles.append(t)
                    mx = t if mx is None else jnp.maximum(mx, t)
                if c1 == i + 1:
                    st["m"] = jnp.max(mx, axis=1, keepdims=True)
                    st["tiles"] = tiles
                yield

        def context(i, st):
            m, tiles = st["m"], st["tiles"]
            o = l = None
            for c0 in range(0, i + 1, PV_TILES):
                c1 = min(c0 + PV_TILES, i + 1)
                ps = [jnp.exp2(t - m) for t in tiles[c0:c1]]
                for p in ps:
                    l = p if l is None else l + p
                if c1 > 1:
                    ps[-1] = jnp.minimum(ps[-1], l)
                pc = jnp.concatenate(ps, axis=1).astype(BF16)
                oc = _dot(pc, v_v[c0 * T:c1 * T, :])
                o = oc if o is None else o + oc
                if c1 == i + 1:
                    l = jnp.sum(l, axis=1, keepdims=True)
                    r = pl.reciprocal(l, approx=True)
                    r = r * (2.0 - l * r)
                    q_v[h, i * T:(i + 1) * T, :] = (o * r).astype(BF16)
                yield

        prev = iter(())
        for i in range(NB - 1, -1, -1):
            st = {}
            cur = scores(i, st)
            for _ in prev:
                next(cur, None)
            _finish(cur)
            if next_head is not None:
                if i < S // PM:
                    k_proj(next_head, i)
                if i + 1 < S // PM:
                    v_proj(next_head, i + 1)
            prev = context(i, st)
        _finish(prev)
        if next_head is not None:
            v_proj(next_head, 0)

    def attend_step(n, carry):
        attend(2 * n, 2 * n + 1)
        attend(2 * n + 1, 2 * n + 2)
        return carry

    lax.fori_loop(0, H // 2 - 1, attend_step, 0)
    attend(H - 2, H - 1)
    attend(H - 1, None)

    wo_copy.wait()

    def out_copy(r):
        return pltpu.make_async_copy(
            o_v.at[r], out_hbm.at[pl.ds(r * RB, RB), :], out_sem.at[r])

    def out_proj(r, carry):
        rows = pl.ds(pl.multiple_of(r * RB, RB), RB)
        ctx = jnp.concatenate([q_v[n, rows, :] for n in range(H)], axis=1)
        b = _dot(ctx, wo_v[...])
        aq = aq_v[rows, :].astype(F32)
        gw = gw_ref[...].astype(F32)
        gw = jnp.concatenate([gw[n:n + 1, :] for n in range(NC)], axis=1)
        g = jax.nn.sigmoid(jnp.sum(aq * gw, axis=1, keepdims=True))
        y = jnp.concatenate([y_v[n, rows, :] for n in range(NC)], axis=1)
        o_v[r] = (g * (aq * y) + (1.0 - g) * b).astype(BF16)
        out_copy(r).start()
        return carry

    lax.fori_loop(0, S // RB, out_proj, 0)
    for r in range(S // RB):
        out_copy(r).wait()


@jax.jit
def pallas_gated_mix__ssm_conv_h3__compressed_kv_cla__prompt_kernel(
    A_q: jax.Array,
    A_k: jax.Array,
    A_v: jax.Array,
    A_shift_k: jax.Array,
    A_ssm_k: jax.Array,
    A_ssm_D: jax.Array,
    B_x: jax.Array,
    B_c_kv: jax.Array,
    B_w_q: jax.Array,
    B_w_uk: jax.Array,
    B_w_uv: jax.Array,
    B_w_o: jax.Array,
    gate_w: jax.Array,
):
    del B_x
    hbm = pl.BlockSpec(memory_space=pl.ANY)
    out = pl.pallas_call(
        _kernel,
        out_shape=jax.ShapeDtypeStruct((S, DM), BF16),
        in_specs=[hbm] * 15,
        out_specs=hbm,
        scratch_shapes=[
            pltpu.VMEM((S, DM), BF16),
            pltpu.VMEM((NC, S + HALO, T), BF16),
            pltpu.VMEM((NC, S, T), BF16),
            pltpu.VMEM((NC, T, S), BF16),
            pltpu.VMEM((S, DC), BF16),
            pltpu.VMEM((2, DM * H // 4, DH), U32),
            pltpu.VMEM((NC, 2, DC // NC * H // 4, DH), U32),
            pltpu.VMEM((NC, 2, DC // NC * H // 4, DH), U32),
            pltpu.VMEM((H * DH, DM), BF16),
            pltpu.VMEM((H, DM + 2 * DC, DH), BF16),
            pltpu.VMEM((H, S, DH), BF16),
            pltpu.VMEM((S, DH), BF16),
            pltpu.VMEM((S, DH), BF16),
            pltpu.VMEM((NC, S, T), F32),
            pltpu.VMEM((S, T), BF16),
            pltpu.VMEM((7 * NB, T, T), F32),
            pltpu.VMEM((S // RB, RB, DM), BF16),
            pltpu.VMEM((2 * T, T), BF16),
            pltpu.VMEM((T, T), BF16),
            pltpu.VMEM((KS, DM), BF16),
            pltpu.VMEM((NC, T), BF16),
            pltpu.VMEM((NC, T), BF16),
            pltpu.VMEM((NC, T), F32),
            pltpu.SMEM((1,), jnp.int32),
            pltpu.SemaphoreType.DMA((5,)),
            pltpu.SemaphoreType.DMA((4,)),
            pltpu.SemaphoreType.DMA((2,)),
            pltpu.SemaphoreType.DMA((3 * NC,)),
            pltpu.SemaphoreType.DMA((4 * NC,)),
            pltpu.SemaphoreType.DMA((3,)),
            pltpu.SemaphoreType.DMA((S // RB,)),
        ],
        compiler_params=pltpu.CompilerParams(vmem_limit_bytes=126 * 2**20),
        name="gated_mix_h3_cla",
    )(
        A_q.reshape(S, DM), A_k.reshape(S, DM), A_v.reshape(S, DM), A_ssm_k,
        B_c_kv.reshape(S, DC), B_w_q, B_w_uk, B_w_uv, B_w_o.reshape(H * DH, DM),
        jnp.zeros((1,), jnp.int32), A_shift_k.T, A_ssm_D.reshape(NC, T), gate_w.reshape(NC, T),
        jnp.asarray(_FWD, BF16), jnp.asarray(_INV, BF16),
    )
    return out.reshape(1, S, DM)
```

```python
import functools
import math

import jax
import jax.numpy as jnp
import numpy as np
from jax import lax
import jax.experimental.pallas as pl
import jax.experimental.pallas.tpu as pltpu

F32 = jnp.float32
BF16 = jnp.bfloat16
U32 = jnp.uint32
P = functools.partial

S = 2048
DM = 1024
H = 32
DH = 128
DC = 512
KS = 4
T = 128
NB = S // T
NC = DM // T
PM = 256
RB = 256
QK_TILES = 4
PV_TILES = 2
X_EDGES = (0, 128, 384, 768, S)
XS, GS, YS = 0, 3 * NB, 6 * NB
HALO = 16


def _dft_matrices():
    even = np.arange(0, T, 2)
    k = np.concatenate([even, T - 1 - even]).astype(np.float64)
    ang = 2.0 * np.pi * np.outer(k + 0.5, np.arange(T)) / (2 * T)
    fwd = np.concatenate([np.cos(ang), -np.sin(ang)], axis=0)
    inv = np.concatenate([np.cos(ang[:T // 2]), -np.sin(ang[:T // 2])], axis=0).T / T
    inv = np.concatenate([inv[0::2], inv[1::2]], axis=0)
    return fwd.astype(np.float32), inv.astype(np.float32)


_FWD, _INV = _dft_matrices()


def _dot(a, b):
    return jnp.dot(a, b, preferred_element_type=F32)


def _dot_nt(a, b):
    return lax.dot_general(a, b, (((1,), (1,)), ((), ())), preferred_element_type=F32)


def _unpack(w):
    return (lax.bitcast_convert_type(w << 16, F32),
            lax.bitcast_convert_type(w & jnp.uint32(0xFFFF0000), F32))


def _split_heads(w):
    lo, hi = _unpack(w)
    return lo.astype(BF16), hi.astype(BF16)


def _finish(gen):
    for _ in gen:
        pass


def _interleave(*streams):
    steps = [((n + 0.5 * (k > 0)) / len(st), k, fn)
             for k, st in enumerate(streams) for n, fn in enumerate(st)]
    for _, _, fn in sorted(steps, key=lambda t: t[:2]):
        fn()


def _kernel(
    aq_hbm, ak_hbm, av_hbm, ssmk_hbm, c_hbm, wq_hbm, wuk_hbm, wuv_hbm, wo_hbm,
    zero_hbm, shift_hbm, ssmd_hbm, gw_hbm, fwd_hbm, inv_hbm,
    out_hbm,
    aq_v, ak_v, av_v, ssmk_v, c_v, wq_raw, wuk_raw, wuv_raw, wo_v,
    w_v, q_v, k_v, v_v, y_v, kv_v, spec_v, o_v,
    fwd_ref, inv_ref, shift_ref, ssmd_ref, gw_ref, ssmd_v, zero_ref,
    small_sem, x_sem, wq_sem, conv_sem, wkv_sem, misc_sem, out_sem,
):
    wr = DC // NC

    def aligned(i, n):
        return pl.ds(i * n if isinstance(i, int) else pl.multiple_of(i * n, n), n)

    def x_copy(n):
        rows = pl.ds(X_EDGES[n], X_EDGES[n + 1] - X_EDGES[n])
        return pltpu.make_async_copy(aq_hbm.at[rows], aq_v.at[rows], x_sem.at[n])

    def wq_copy(g):
        pairs = H // 4
        return pltpu.make_async_copy(
            wq_hbm.bitcast(U32).at[:, pl.ds(g * pairs, pairs), :],
            wq_raw.at[g].reshape(DM, pairs, DH), wq_sem.at[g])

    def conv_copies(ct):
        ch = aligned(ct, T)
        return (
            pltpu.make_async_copy(ak_hbm.at[:, ch], ak_v.at[ct, pl.ds(HALO, S)], conv_sem.at[3 * ct]),
            pltpu.make_async_copy(av_hbm.at[:, ch], av_v.at[ct], conv_sem.at[3 * ct + 1]),
            pltpu.make_async_copy(ssmk_hbm.at[ch], ssmk_v.at[ct], conv_sem.at[3 * ct + 2]),
        )

    def wkv_copies(ct):
        pairs = H // 4
        return tuple(
            pltpu.make_async_copy(
                src.bitcast(U32).at[aligned(ct, wr), pl.ds(g * pairs, pairs), :],
                dst.at[ct, g].reshape(wr, pairs, DH), wkv_sem.at[4 * ct + 2 * n + g])
            for n, (src, dst) in enumerate(((wuk_hbm, wuk_raw), (wuv_hbm, wuv_raw)))
            for g in range(2))

    c_copy = pltpu.make_async_copy(c_hbm, c_v, misc_sem.at[0])
    wo_copy = pltpu.make_async_copy(wo_hbm, wo_v, misc_sem.at[1])

    small_copies = [
        pltpu.make_async_copy(src, dst, small_sem.at[n]) for n, (src, dst) in enumerate((
            (shift_hbm, shift_ref), (ssmd_hbm, ssmd_ref), (gw_hbm, gw_ref),
            (fwd_hbm, fwd_ref), (inv_hbm, inv_ref)))]
    zero_copy = pltpu.make_async_copy(zero_hbm, zero_ref, misc_sem.at[2])

    zero_copy.start()
    wq_copy(0).start()
    x_copy(0).start()
    ak_v[:, 0:HALO, :] = jnp.zeros((NC, HALO, T), BF16)
    zero_copy.wait()

    qscale = DH ** -0.5 * math.log2(math.e)
    zero = zero_ref[0]

    def unpack_wq(pair, part):
        g, p = divmod(pair, H // 4)
        lo, hi = _split_heads(wq_raw[g, pl.ds(part * T * (H // 4) + p, T, stride=H // 4), :])
        w_v[zero + 2 * pair, part * T:(part + 1) * T, :] = lo
        w_v[zero + 2 * pair + 1, part * T:(part + 1) * T, :] = hi

    def unpack_wkv(ct, pair):
        k_rows, v_rows = aligned(DM // wr + ct, wr), aligned((DM + DC) // wr + ct, wr)
        g, p = divmod(pair, H // 4)
        k0, k1 = _split_heads(wuk_raw[ct, g, pl.ds(p, wr, stride=H // 4), :])
        v0, v1 = _split_heads(wuv_raw[ct, g, pl.ds(p, wr, stride=H // 4), :])
        w_v[2 * pair, k_rows, :] = k0
        w_v[2 * pair + 1, k_rows, :] = k1
        w_v[2 * pair, v_rows, :] = v0
        w_v[2 * pair + 1, v_rows, :] = v1

    def q_proj(h, r, n):
        rows = aligned(r, n)
        q_v[h, rows, :] = (_dot(aq_v[rows, :], w_v[h, :DM, :]) * qscale).astype(BF16)

    def k_proj(h, r):
        rows = slice(r * PM, (r + 1) * PM)
        k_v[rows, :] = _dot(c_v[rows, :], w_v[h, DM:DM + DC, :]).astype(BF16)

    def v_proj(h, r):
        rows = slice(r * PM, (r + 1) * PM)
        v_v[rows, :] = _dot(c_v[rows, :], w_v[h, DM + DC:, :]).astype(BF16)

    def conv_input(ct, i):
        sh = shift_ref[:, aligned(ct, T)].astype(F32)
        kf = ak_v[ct, i * T:(i + 1) * T + HALO, :].astype(F32)
        ksh = kf * sh[0:1, :]
        for j in range(1, KS):
            ksh = ksh + pltpu.roll(kf, j, 0) * sh[j:j + 1, :]
        rows = slice(i * T, (i + 1) * T)
        kv_v[rows, :] = (ksh[HALO:] * av_v[ct, rows, :].astype(F32)).astype(BF16)

    def input_spectrum(i):
        xf = _dot(fwd_ref[...], kv_v[i * T:(i + 1) * T, :])
        spec_v[XS + i] = xf[:T] + xf[T:]
        spec_v[XS + NB + i] = xf[:T]
        spec_v[XS + 2 * NB + i] = xf[T:]

    def kernel_spectrum(ct, i, prev):
        half = T // 2
        hf = _dot_nt(fwd_ref[...], ssmk_v[ct, :, i * T:(i + 1) * T])
        gr, gi = hf[:T], hf[T:]
        if i:
            pr, pi = prev[0][:T], prev[0][T:]
            gr = jnp.concatenate([gr[:half] - pi[:half], gr[half:] + pi[half:]], axis=0)
            gi = jnp.concatenate([gi[:half] + pr[:half], gi[half:] - pr[half:]], axis=0)
        prev[0] = hf
        spec_v[GS + i] = gr
        spec_v[GS + NB + i] = gi - gr
        spec_v[GS + 2 * NB + i] = gi + gr

    def conv_bins(lo, hi, f):
        rows = slice(8 * f, 8 * f + 8)

        def part(n):
            outs = [None] * (hi - lo)
            for j in range(hi):
                g = spec_v[GS + n * NB + j, rows, :]
                for i in range(max(lo, j), hi):
                    t = spec_v[XS + n * NB + i - j, rows, :] * g
                    outs[i - lo] = t if j == 0 else outs[i - lo] + t
            return outs

        s1 = part(0)
        re = [a - b for a, b in zip(s1, part(2))]
        im = [a + b for a, b in zip(s1, part(1))]
        base = YS + (zero if f % 4 == 3 else 0)
        for i in range(lo, hi):
            spec_v[base + 2 * i, rows, :] = re[i - lo]
            spec_v[base + 2 * i + 1, rows, :] = im[i - lo]

    def conv_inverse(ct, i):
        d = ssmd_v[pl.ds(ct, 1), :]
        half = T // 2
        re, im = spec_v[YS + 2 * i], spec_v[YS + 2 * i + 1]
        folded = (jnp.concatenate([re[:half] + re[half:], im[:half] - im[half:]], axis=0),
                  jnp.concatenate([re[:half] - re[half:], im[:half] + im[half:]], axis=0))
        kv = _unpack(pltpu.bitcast(kv_v[i * T:(i + 1) * T, :], U32))
        for odd in range(2):
            y = _dot(inv_ref[odd * half:(odd + 1) * half, :], folded[odd].astype(BF16))
            y_v[ct, pl.ds(i * T + odd, half, stride=2), :] = y + kv[odd] * d

    def conv_tile(ct, fillers):
        slots = (0, 3, 7, 13, 20, len(fillers))
        inputs = (0, 6, 12, NB, NB, NB)
        prev = [None]
        for r in range(-1, 4):
            new = range(inputs[r + 1], inputs[r + 2])
            side = [P(conv_input, ct, i) for i in new]
            for i in new:
                side.append(P(input_spectrum, i))
                if r < 0:
                    side += [P(kernel_spectrum, ct, j, prev)
                             for j in range(i * NB // len(new), (i + 1) * NB // len(new))]
            if r > 0:
                side += [P(conv_inverse, ct, i) for i in range(4 * r - 4, 4 * r)]
            bins, unpack = [], []
            if r >= 0:
                bins = [P(conv_bins, 4 * r, 4 * r + 4, f) for f in range(T // 8)]
                unpack = [P(unpack_wkv, ct, pair) for pair in range(4 * r, 4 * r + 4)]
            _interleave(fillers[slots[r + 1]:slots[r + 2]], bins, side, unpack)
        for i in range(NB - 4, NB):
            conv_inverse(ct, i)

    after_x = ((x_copy(1), x_copy(2)),
               (x_copy(3), *small_copies),
               conv_copies(0) + wkv_copies(0))
    parts = range(DM // T)
    wq_copy(0).wait()
    for n in range(3):
        x_copy(n).wait()
        for cp in after_x[n]:
            cp.start()
        steps = []
        for h in range(8):
            if n == 0 and h % 2 == 0:
                steps += [P(unpack_wq, h // 2, part) for part in parts]
            steps += [P(q_proj, h, r, T) for r in range(X_EDGES[n] // T, X_EDGES[n + 1] // T)]
        _interleave(steps, [P(unpack_wq, pair, part)
                            for pair in ((), (4, 5), (6, 7))[n] for part in parts])
    x_copy(3).wait()
    for cp in small_copies:
        cp.wait()
    ssmd_v[...] = ssmd_ref[...].astype(F32)
    chunks, first = S // PM, 4
    per_tile = (H * chunks - 8 * first) // NC

    def q_step(ct, carry):
        for cp in conv_copies(ct) + wkv_copies(ct):
            cp.wait()

        @pl.when(ct + 1 < NC)
        def _():
            for cp in conv_copies(ct + 1) + wkv_copies(ct + 1):
                cp.start()

        @pl.when(ct == 0)
        def _():
            wq_copy(1).start()

        @pl.when(ct == 2)
        def _():
            wq_copy(1).wait()
            c_copy.start()
            _interleave([P(q_proj, h, r, T) for h in range(8) for r in (6, 7)],
                        [P(unpack_wq, pair, part) for pair in range(8, 16) for part in parts])

        def piece(n):
            p = per_tile * ct + n
            early = p < 8 * (chunks - first)
            h = jnp.where(early, p % 8, (p + 8 * first) // chunks)
            r = jnp.where(early, first + p // 8, p % chunks)
            q_proj(h, r, PM)

        conv_tile(ct, [P(piece, n) for n in range(per_tile)])
        return carry

    lax.fori_loop(0, NC, q_step, 0)
    c_copy.wait()
    wo_copy.start()
    for r in range(S // PM):
        k_proj(0, r)
        v_proj(0, r)

    def attend(h, next_head):
        tri = (lax.broadcasted_iota(jnp.int32, (T, T), 1)
               <= lax.broadcasted_iota(jnp.int32, (T, T), 0))

        def scores(i, st):
            q = q_v[h, i * T:(i + 1) * T, :]
            tiles, mx = [], None
            for c0 in range(0, i + 1, QK_TILES):
                c1 = min(c0 + QK_TILES, i + 1)
                s = _dot_nt(q, k_v[c0 * T:c1 * T, :])
                for j in range(c0, c1):
                    t = s[:, (j - c0) * T:(j - c0 + 1) * T]
                    if j == i:
                        t = jnp.where(tri, t, -1e9)
                    tiles.append(t)
                    mx = t if mx is None else jnp.maximum(mx, t)
                if c1 == i + 1:
                    st["m"] = jnp.max(mx, axis=1, keepdims=True)
                    st["tiles"] = tiles
                yield

        def context(i, st):
            m, tiles = st["m"], st["tiles"]
            o = l = None
            for c0 in range(0, i + 1, PV_TILES):
                c1 = min(c0 + PV_TILES, i + 1)
                ps = [jnp.exp2(t - m) for t in tiles[c0:c1]]
                for p in ps:
                    l = p if l is None else l + p
                if c1 > 1:
                    ps[-1] = jnp.minimum(ps[-1], l)
                pc = jnp.concatenate(ps, axis=1).astype(BF16)
                oc = _dot(pc, v_v[c0 * T:c1 * T, :])
                o = oc if o is None else o + oc
                if c1 == i + 1:
                    l = jnp.sum(l, axis=1, keepdims=True)
                    r = pl.reciprocal(l, approx=True)
                    r = r * (2.0 - l * r)
                    q_v[h, i * T:(i + 1) * T, :] = (o * r).astype(BF16)
                yield

        prev = iter(())
        for i in range(NB - 1, -1, -1):
            st = {}
            cur = scores(i, st)
            for _ in prev:
                next(cur, None)
            _finish(cur)
            if next_head is not None:
                if i < S // PM:
                    k_proj(next_head, i)
                if i + 1 < S // PM:
                    v_proj(next_head, i + 1)
            prev = context(i, st)
        _finish(prev)
        if next_head is not None:
            v_proj(next_head, 0)

    def attend_step(n, carry):
        attend(2 * n, 2 * n + 1)
        attend(2 * n + 1, 2 * n + 2)
        return carry

    lax.fori_loop(0, H // 2 - 1, attend_step, 0)
    attend(H - 2, H - 1)
    attend(H - 1, None)

    wo_copy.wait()

    def out_copy(r):
        return pltpu.make_async_copy(
            o_v.at[r], out_hbm.at[pl.ds(r * RB, RB), :], out_sem.at[r])

    def out_proj(r, carry):
        rows = pl.ds(pl.multiple_of(r * RB, RB), RB)
        ctx = jnp.concatenate([q_v[n, rows, :] for n in range(H)], axis=1)
        b = _dot(ctx, wo_v[...])
        aq = aq_v[rows, :].astype(F32)
        gw = gw_ref[...].astype(F32)
        gw = jnp.concatenate([gw[n:n + 1, :] for n in range(NC)], axis=1)
        g = jax.nn.sigmoid(jnp.sum(aq * gw, axis=1, keepdims=True))
        y = jnp.concatenate([y_v[n, rows, :] for n in range(NC)], axis=1)
        o_v[r] = (g * (aq * y) + (1.0 - g) * b).astype(BF16)
        out_copy(r).start()
        return carry

    lax.fori_loop(0, S // RB, out_proj, 0)
    for r in range(S // RB):
        out_copy(r).wait()


@jax.jit
def pallas_gated_mix__ssm_conv_h3__compressed_kv_cla__prompt_kernel(
    A_q: jax.Array,
    A_k: jax.Array,
    A_v: jax.Array,
    A_shift_k: jax.Array,
    A_ssm_k: jax.Array,
    A_ssm_D: jax.Array,
    B_x: jax.Array,
    B_c_kv: jax.Array,
    B_w_q: jax.Array,
    B_w_uk: jax.Array,
    B_w_uv: jax.Array,
    B_w_o: jax.Array,
    gate_w: jax.Array,
):
    del B_x
    hbm = pl.BlockSpec(memory_space=pl.ANY)
    out = pl.pallas_call(
        _kernel,
        out_shape=jax.ShapeDtypeStruct((S, DM), BF16),
        in_specs=[hbm] * 15,
        out_specs=hbm,
        scratch_shapes=[
            pltpu.VMEM((S, DM), BF16),
            pltpu.VMEM((NC, S + HALO, T), BF16),
            pltpu.VMEM((NC, S, T), BF16),
            pltpu.VMEM((NC, T, S), BF16),
            pltpu.VMEM((S, DC), BF16),
            pltpu.VMEM((2, DM * H // 4, DH), U32),
            pltpu.VMEM((NC, 2, DC // NC * H // 4, DH), U32),
            pltpu.VMEM((NC, 2, DC // NC * H // 4, DH), U32),
            pltpu.VMEM((H * DH, DM), BF16),
            pltpu.VMEM((H, DM + 2 * DC, DH), BF16),
            pltpu.VMEM((H, S, DH), BF16),
            pltpu.VMEM((S, DH), BF16),
            pltpu.VMEM((S, DH), BF16),
            pltpu.VMEM((NC, S, T), F32),
            pltpu.VMEM((S, T), BF16),
            pltpu.VMEM((8 * NB, T, T), F32),
            pltpu.VMEM((S // RB, RB, DM), BF16),
            pltpu.VMEM((2 * T, T), BF16),
            pltpu.VMEM((T, T), BF16),
            pltpu.VMEM((KS, DM), BF16),
            pltpu.VMEM((NC, T), BF16),
            pltpu.VMEM((NC, T), BF16),
            pltpu.VMEM((NC, T), F32),
            pltpu.SMEM((1,), jnp.int32),
            pltpu.SemaphoreType.DMA((5,)),
            pltpu.SemaphoreType.DMA((4,)),
            pltpu.SemaphoreType.DMA((2,)),
            pltpu.SemaphoreType.DMA((3 * NC,)),
            pltpu.SemaphoreType.DMA((4 * NC,)),
            pltpu.SemaphoreType.DMA((3,)),
            pltpu.SemaphoreType.DMA((S // RB,)),
        ],
        compiler_params=pltpu.CompilerParams(vmem_limit_bytes=126 * 2**20),
        name="gated_mix_h3_cla",
    )(
        A_q.reshape(S, DM), A_k.reshape(S, DM), A_v.reshape(S, DM), A_ssm_k,
        B_c_kv.reshape(S, DC), B_w_q, B_w_uk, B_w_uv, B_w_o.reshape(H * DH, DM),
        jnp.zeros((1,), jnp.int32), A_shift_k.T, A_ssm_D.reshape(NC, T), gate_w.reshape(NC, T),
        jnp.asarray(_FWD, BF16), jnp.asarray(_INV, BF16),
    )
    return out.reshape(1, S, DM)
```
